```python
import os as _os
_os.environ.setdefault("JAX_PLATFORMS", "cpu")
import jax
import jax.numpy as jnp

def _softmax(x, axis=-1):
    return jax.nn.softmax(x, axis=axis)
def _gelu(x):
    return jax.nn.gelu(x, approximate=True)
def _silu(x):
    return jax.nn.silu(x)
def _sigmoid(x):
    return jax.nn.sigmoid(x)
def _layernorm(x, axis=-1, eps=1e-5):
    m = jnp.mean(x, axis=axis, keepdims=True)
    v = jnp.var(x, axis=axis, keepdims=True)
    return (x - m) / jnp.sqrt(v + eps)
def _scatter_add(tgt, idx, src, axis=0):
    return tgt.at[idx].add(src)
def _segment_sum(src, seg, n):
    return jax.ops.segment_sum(src, seg, n)
class _Rng:
    def __init__(self, key):
        self._k = key
    def _next(self):
        self._k, sub = jax.random.split(self._k)
        return sub
    def normal(self, shape):
        return jax.random.normal(self._next(), shape, dtype=jnp.bfloat16)
    def randint(self, lo, hi, shape):
        return jax.random.randint(self._next(), shape, lo, hi, dtype=jnp.int32)
    def uniform(self, shape, lo=0.0, hi=1.0):
        return jax.random.uniform(self._next(), shape, jnp.bfloat16, lo, hi)
    def permutation(self, n):
        return jax.random.permutation(self._next(), n)


kernel_name = 'gated_mix__softmax_full_mha__dense_activation_squared_relu__prompt'

def setup_inputs():
    _rng = _Rng(jax.random.key(int.from_bytes(__import__("os").urandom(4), "little")))
    _w = (lambda a: (lambda t: t.astype(jnp.bfloat16) if jnp.issubdtype(t.dtype, jnp.floating) else t)(jnp.asarray(a)))
    def _A_setup():
        B, S, D = 1, 2048, 640
        return {
            "x": _w((lambda *s: _rng.normal(s) * 0.05)(B, S, D)),
            "wqkv": _w((lambda *s: _rng.normal(s) * 0.4)(D, 3 * D)),
            "wo": _w((lambda *s: _rng.normal(s) * 0.05)(D, D)),
        }
    _A_in = _A_setup()

    def _B_setup():
        B, S, D, F = 1, 2048, 640, 1536
        return {
            "x": _w((lambda *s: _rng.normal(s) * 0.05)(B, S, D)),
            "w1": _w((lambda *s: _rng.normal(s) * 0.05)(D, F)),
            "b1": _w((lambda *s: _rng.normal(s) * 0.05)(F)),
            "w2": _w((lambda *s: _rng.normal(s) * 0.05)(F, D)),
            "b2": _w((lambda *s: _rng.normal(s) * 0.05)(D)),
        }
    _B_in = _B_setup()

    return {
        "A_x": _A_in["x"],
        "A_wqkv": _A_in["wqkv"],
        "A_wo": _A_in["wo"],
        "B_x": _B_in["x"],
        "B_w1": _B_in["w1"],
        "B_b1": _B_in["b1"],
        "B_w2": _B_in["w2"],
        "B_b2": _B_in["b2"],
        "gate_w": _w((lambda *s: _rng.normal(s) * 0.05)(640) * 16.0),
    }

def reference(A_x, A_wqkv, A_wo, B_x, B_w1, B_b1, B_w2, B_b2, gate_w):
    def _A_ref(x, wqkv, wo):
        B, S, D = x.shape
        H = 32; Dh = D // H
        qkv = (lambda x, *d: x.transpose(*d))((x @ wqkv).reshape(B, S, 3, H, Dh), 2, 0, 3, 1, 4)
        q, k, v = qkv[0], qkv[1], qkv[2]
        scale = Dh ** -0.5
        scores = jnp.einsum("bhqd,bhkd->bhqk", q, k) * scale
        p = _softmax(scores, axis=-1)
        o = jnp.einsum("bhqk,bhkd->bhqd", p, v)
        return (lambda x, *d: x.transpose(*d))(o, 0, 2, 1, 3).reshape(B, S, D) @ wo

    def _B_ref(x, w1, b1, w2, b2):
        h = jnp.einsum("bsd,df->bsf", x, w1) + b1
        zero = jnp.zeros_like(h)
        r = jnp.where(h > zero, h, zero)
        h = r * r
        out = jnp.einsum("bsf,fd->bsd", h, w2) + b2
        return out

    x = A_x
    g = _sigmoid((x * gate_w).sum(-1, keepdims=True))
    a = _A_ref(x, A_wqkv, A_wo)
    b = _B_ref(x, B_w1, B_b1, B_w2, B_b2)
    return g * a + (1 - g) * b
```

```python
import functools
import math
import jax
import jax.numpy as jnp
from jax import lax
import jax.experimental.pallas as pl
import jax.experimental.pallas.tpu as pltpu

S, D, H, DH, F = 2048, 640, 32, 20, 1536
NSLAB = 9
BF = jnp.bfloat16
F32 = jnp.float32


def _make_kernel(TQ=512, C=128, UNROLL=2):
    NQ = S // TQ
    NC = S // C
    QSCALE = (DH ** -0.5) * math.log2(math.e)

    def kernel(x_ref, wqkv_ref, wo_ref, w1_ref, b1_ref, w2_ref, b2_ref, gw_ref, o_ref,
               wqvT_ref, k_ref, qT_ref, vT_ref, sa_ref, sb_ref, oT_ref):
        qi = pl.program_id(0)

        @pl.when(qi == 0)
        def _proj():
            wqvT_ref[0:D, :] = wqkv_ref[:, 0:D].T
            wqvT_ref[D:2 * D, :] = wqkv_ref[:, 2 * D:3 * D].T

            def body(t, carry):
                r0 = pl.multiple_of(t * TQ, TQ)
                xt = x_ref[pl.ds(r0, TQ), :]
                k = jnp.dot(xt, wqkv_ref[:, D:2 * D], preferred_element_type=F32)
                lane = lax.broadcasted_iota(jnp.int32, (TQ, 128), 1)
                for j in range(5):
                    k_ref[j, pl.ds(r0, TQ), :] = k[:, 128 * j:128 * j + 128].astype(BF)
                for j in range(4):
                    k_ref[5 + j, pl.ds(r0, TQ), :] = jnp.where(
                        lane >= 64, k[:, 128 * j:128 * j + 128], k[:, 128 * j + 128:128 * j + 256]).astype(BF)
                qv = lax.dot_general(wqvT_ref[...], xt, (((1,), (1,)), ((), ())), preferred_element_type=F32)
                q = (qv[:D] * QSCALE).astype(BF)
                for j in range(5):
                    qT_ref[t, j] = q[128 * j:128 * j + 128]
                for j in range(4):
                    qT_ref[t, 5 + j, 0:64, :] = q[128 * j + 128:128 * j + 192]
                    qT_ref[t, 5 + j, 64:128, :] = q[128 * j + 64:128 * j + 128]
                vT_ref[t] = qv[D:].astype(BF)
                return carry

            lax.fori_loop(0, NQ, body, 0)

        def slab_of(h):
            r = h * DH
            j = r // 128
            return jnp.where((r % 128) > 108, j + 5, j)

        def load_qm(h):
            sl = slab_of(h)
            qw = pltpu.bitcast(qT_ref[qi, sl], jnp.int32)
            row = lax.broadcasted_iota(jnp.int32, (64, TQ), 0) * 2
            rel = (row - h * DH) & 127
            qm = jnp.where(rel < DH, qw, 0)
            return sl, pltpu.bitcast(qm, BF)

        def step(h_next, h_cur, s_next, s_cur, m_cur):
            if h_next is not None:
                sl, qm = load_qm(h_next)
                mx = None
            if h_cur is not None:
                w = pl.multiple_of(((h_cur * DH) // 16) * 16, 16)
                off = h_cur * DH - w
                rowp = lax.broadcasted_iota(jnp.int32, (16, C), 0) * 2
                usedp = (rowp >= off) & (rowp < off + DH)
                ones2 = jnp.full((16, C), 0x3F803F80, jnp.int32)
                acc = None
            for c in range(NC):
                if h_next is not None:
                    s = jnp.dot(k_ref[sl, c * C:(c + 1) * C, :], qm, preferred_element_type=F32)
                    s_next[c * C:(c + 1) * C, :] = s
                    cm = jnp.max(s.reshape(C // 8, 8, TQ), axis=0)
                    mx = cm if mx is None else jnp.maximum(mx, cm)
                if h_cur is not None:
                    p = jnp.exp2(s_cur[c * C:(c + 1) * C, :] - m_cur).astype(BF)
                    t, lo = (c * C) // TQ, (c * C) % TQ
                    vw = pltpu.bitcast(vT_ref[t, pl.ds(w, 32), lo:lo + C], jnp.int32)
                    vw = pltpu.bitcast(jnp.where(usedp, vw, ones2), BF)
                    pv = jnp.dot(vw, p, preferred_element_type=F32)
                    acc = pv if acc is None else acc + pv
            if h_cur is not None:
                l = jnp.where(off == 12, acc[0:1], acc[31:32])
                on = acc * (1.0 / l)
                row = lax.broadcasted_iota(jnp.int32, (32, TQ), 0)
                used = (row >= off) & (row < off + DH)
                pltpu.store(oT_ref.at[pl.ds(w, 32), :], on, mask=used)
            if h_next is not None:
                return jnp.max(mx, axis=0, keepdims=True)
            return None

        bufs = (sa_ref, sb_ref)
        m0 = step(0, None, sa_ref, None, None)

        def loop_body(i, m):
            h = i * UNROLL
            for u in range(UNROLL):
                m = step(h + u + 1, h + u, bufs[(u + 1) % 2], bufs[u % 2], m)
            return m

        n_full = (H - 1) // UNROLL
        m = lax.fori_loop(0, n_full, loop_body, m0)
        for h in range(n_full * UNROLL, H - 1):
            m = step(h + 1, h, bufs[(h + 1) % 2], bufs[h % 2], m)
        step(None, H - 1, None, bufs[(H - 1) % 2], m)

        r0 = pl.multiple_of(qi * TQ, TQ)
        xt = x_ref[pl.ds(r0, TQ), :]
        o = oT_ref[...].T.astype(BF)
        a = jnp.dot(o, wo_ref[...], preferred_element_type=F32)
        hh = jnp.dot(xt, w1_ref[...], preferred_element_type=F32) + b1_ref[...].astype(F32)
        r = jnp.maximum(hh, 0.0)
        hh = (r * r).astype(BF)
        b = jnp.dot(hh, w2_ref[...], preferred_element_type=F32) + b2_ref[...].astype(F32)
        z = jnp.sum(xt.astype(F32) * gw_ref[...].astype(F32), axis=-1, keepdims=True)
        g = jax.nn.sigmoid(z)
        o_ref[...] = (g * a + (1.0 - g) * b).astype(o_ref.dtype)

    def full(shape):
        return pl.BlockSpec(shape, lambda i: (0,) * len(shape))

    @jax.jit
    def fn(A_x, A_wqkv, A_wo, B_x, B_w1, B_b1, B_w2, B_b2, gate_w):
        x = A_x.reshape(S, D)
        out = pl.pallas_call(
            kernel,
            grid=(NQ,),
            in_specs=[full((S, D)), full((D, 3 * D)), full((D, D)), full((D, F)), full((1, F)),
                      full((F, D)), full((1, D)), full((1, D))],
            out_specs=pl.BlockSpec((TQ, D), lambda i: (i, 0)),
            out_shape=jax.ShapeDtypeStruct((S, D), BF),
            scratch_shapes=[
                pltpu.VMEM((2 * D, D), BF),
                pltpu.VMEM((NSLAB, S, 128), BF),
                pltpu.VMEM((NQ, NSLAB, 128, TQ), BF),
                pltpu.VMEM((NQ, D, TQ), BF),
                pltpu.VMEM((S, TQ), F32),
                pltpu.VMEM((S, TQ), F32),
                pltpu.VMEM((D, TQ), F32),
            ],
            compiler_params=pltpu.CompilerParams(
                dimension_semantics=("arbitrary",), vmem_limit_bytes=100 * 1024 * 1024),
            name="gmix",
        )(x, A_wqkv, A_wo, B_w1, B_b1.reshape(1, F), B_w2, B_b2.reshape(1, D), gate_w.reshape(1, D))
        return out.reshape(1, S, D)

    return fn


_impl = _make_kernel()


@jax.jit
def pallas_gated_mix__softmax_full_mha__dense_activation_squared_relu__prompt_kernel(
    A_x, A_wqkv, A_wo, B_x, B_w1, B_b1, B_w2, B_b2, gate_w):
    return _impl(A_x, A_wqkv, A_wo, B_x, B_w1, B_b1, B_w2, B_b2, gate_w)
```

```python
import contextlib
import math
import jax
import jax.numpy as jnp
from jax import lax
import jax.experimental.pallas as pl
import jax.experimental.pallas.tpu as pltpu

S, D, H, DH, F = 2048, 640, 32, 20, 1536
VR = 24
BF = jnp.bfloat16
F32 = jnp.float32
I32 = jnp.int32


def _make_kernel(TE=256, GH=4, NH=2, NS=16, SH=1, FORCE=None, TBOUND=60.0, SCOPES=False, KSUB=128, X0=512):
    TQ = 512
    C = 128
    NQ = S // TQ
    NC = S // C
    NE = S // TE
    NL = TQ // 128
    NGRP = H // GH
    TF = S // NGRP
    R = 16 * NC
    RG = R // 8
    QSCALE = (DH ** -0.5) * math.log2(math.e)
    XCH = [(0, X0), (X0, 1024), (1024, S)] if X0 < 1024 else [(0, 1024), (1024, S)]
    NX = len(XCH)

    def scope(name):
        return jax.named_scope(name) if SCOPES else contextlib.nullcontext()

    def kernel(x_hbm, wqkv_hbm, wo_hbm, w1_hbm, b1_hbm, w2_hbm, b2_hbm, gw_hbm, o_hbm,
               x_ref, wqkv_ref, wo_ref, w1_ref, w2_ref, o_ref,
               wqvT_ref, kn_ref, k_ref, qp_ref, q32_ref, vT_ref, oT_ref, c_ref, g_ref,
               kf_ref, kb_ref, qb_ref, s_ref, qmax_ref, kmax_ref, vmax_ref, b1_ref, b2_ref, gw_ref, z_ref,
               sem_in, sem_out):
        def cp_x(i):
            lo, hi = XCH[i]
            return pltpu.make_async_copy(x_hbm.at[0, pl.ds(lo, hi - lo), :], x_ref.at[pl.ds(lo, hi - lo), :], sem_in.at[i])

        def cp_w(j):
            return pltpu.make_async_copy(wqkv_hbm.at[:, pl.ds(j * D, D)], wqkv_ref.at[j], sem_in.at[NX + j])

        late = [pltpu.make_async_copy(src, dst, sem_in.at[NX + 3 + i])
                for i, (src, dst) in enumerate([(w1_hbm, w1_ref), (w2_hbm, w2_ref), (wo_hbm, wo_ref),
                                                (b1_hbm, b1_ref), (b2_hbm, b2_ref), (gw_hbm, gw_ref)])]
        cp_x(0).start()
        cp_w(1).start()
        for i in range(1, NX - 1):
            cp_x(i).start()
        cp_w(0).start()
        cp_w(2).start()
        cp_x(NX - 1).start()
        for c in late:
            c.start()

        def lane_window(slabs, start, lane):
            j, o = divmod(start, 128)
            if o == 0:
                return slabs[j]
            a = slabs[j]
            if j + 1 < len(slabs):
                a = jnp.where(lane >= o, a, slabs[j + 1])
            return pltpu.roll(a, 128 - o, 1)

        def kproj(lo, hi):
            km = None
            for r in range(lo, hi, KSUB):
                k = jnp.dot(x_ref[r:r + KSUB, :], wqkv_ref[1], preferred_element_type=F32)
                kn_ref[r // 2:(r + KSUB) // 2, :] = pltpu.bitcast(k.astype(BF), I32)
                kr = jnp.max(jnp.abs(k).reshape(KSUB // 8, 8, D), axis=0)
                km = kr if km is None else jnp.maximum(km, kr)
                ks = jnp.concatenate([k[i * 128:i * 128 + 16] for i in range(KSUB // 128)], axis=0)
                nr = ks.shape[0]
                slabs = [ks[:, 128 * j:128 * j + 128] for j in range(5)]
                lane = lax.broadcasted_iota(I32, (nr, 128), 1)
                for gi in range(NGRP):
                    kf_ref[gi, r // 8:r // 8 + nr, :] = lane_window(slabs, gi * GH * DH, lane)
            kmax_ref[...] = km if lo == 0 else jnp.maximum(kmax_ref[...], km)

        with scope("wait0"):
            cp_x(0).wait()
            cp_w(1).wait()
        with scope("kproj"):
            kproj(*XCH[0])
            for i in range(1, NX - 1):
                cp_x(i).wait()
                kproj(*XCH[i])
            cp_w(0).wait()
            cp_w(2).wait()
            cp_x(NX - 1).wait()
            kproj(*XCH[NX - 1])
            wqvT_ref[0:D, :] = wqkv_ref[0].T
            wqvT_ref[D:2 * D, :] = wqkv_ref[2].T
            qmax_ref[...] = jnp.zeros_like(qmax_ref)
            vmax_ref[...] = jnp.zeros_like(vmax_ref)

        def qvproj(t, carry):
            r0 = pl.multiple_of(t * TQ, TQ)
            xt = x_ref[pl.ds(r0, TQ), :]
            qv = lax.dot_general(wqvT_ref[...], xt, (((1,), (1,)), ((), ())), preferred_element_type=F32)
            qf = qv[:D] * QSCALE
            q32_ref[t] = qf
            qa = jnp.abs(qf)
            qm = qmax_ref[...]
            for j in range(NL):
                qm = jnp.maximum(qm, qa[:, 128 * j:128 * j + 128])
            qmax_ref[...] = qm
            v = qv[D:]
            vmax_ref[...] = jnp.maximum(vmax_ref[...], jnp.max(jnp.abs(v).reshape(D // 8, 8, TQ), axis=0))
            row = lax.broadcasted_iota(I32, (VR, TQ), 0)
            zpad = jnp.zeros((32 - VR, TQ), F32)
            for h in range(H):
                off = 4 * (h % 2)
                w = h * DH - off
                used = (row >= off) & (row < off + DH)
                qw = jnp.concatenate([jnp.where(used, qf[w:w + VR], 0.0), zpad], axis=0)
                qp_ref[t, h] = pltpu.bitcast(qw.astype(BF), I32)
                vT_ref[t, h] = jnp.where(used, v[w:w + VR], 1.0)
            rk = pl.multiple_of(t * (TQ // 2), TQ // 2)
            kn = kn_ref[pl.ds(rk, TQ // 2), :]
            slabs = [kn[:, 128 * j:128 * j + 128] for j in range(5)]
            lane = lax.broadcasted_iota(I32, (TQ // 2, 128), 1)
            for h in range(H):
                w = h * DH - 4 * (h % 2)
                j, o = divmod(w, 128)
                sl = slabs[j:j + 2] if o + 32 > 128 else slabs[j:j + 1]
                k_ref[h, pl.ds(rk, TQ // 2), :] = lane_window(sl, o, lane)
            return carry

        with scope("qvproj"):
            lax.fori_loop(0, NQ, qvproj, 0)

        with scope("guard"):
            qa = jnp.max(qmax_ref[...], axis=1, keepdims=True)
            rel = lax.broadcasted_iota(I32, (D, 128), 0) - DH * lax.broadcasted_iota(I32, (D, 128), 1)
            qn2 = jnp.sum(jnp.where((rel >= 0) & (rel < DH), qa * qa, 0.0), axis=0, keepdims=True)
            qn2 = jnp.max(qn2, axis=1, keepdims=True)
            ka = jnp.max(kmax_ref[...], axis=0, keepdims=True)
            rel = lax.broadcasted_iota(I32, (H, D), 1) - DH * lax.broadcasted_iota(I32, (H, D), 0)
            kn2 = jnp.sum(jnp.where((rel >= 0) & (rel < DH), ka * ka, 0.0), axis=1, keepdims=True)
            kn2 = jnp.max(kn2, axis=0, keepdims=True)
            vm = jnp.max(jnp.max(vmax_ref[...], axis=0, keepdims=True), axis=1, keepdims=True)
            safe = (qn2 * kn2 <= TBOUND * TBOUND) & (vm <= 2.0 ** 40) & (vm >= 2.0 ** -40)
            unsafe = jnp.max(jnp.where(safe, 0, 1).astype(I32))
            if FORCE is not None:
                unsafe = jnp.maximum(unsafe, FORCE)
            z_ref[0] = unsafe
            for c in late:
                c.wait()

        def finish(h, odd, qb, acc):
            off = odd * 4
            if isinstance(odd, int):
                l = acc[0:1] if odd else acc[VR - 1:VR]
            else:
                l = jnp.where(odd == 1, acc[0:1], acc[VR - 1:VR])
            on = acc * (1.0 / l)
            row = lax.broadcasted_iota(I32, (VR, TQ), 0)
            used = (row >= off) & (row < off + DH)
            pltpu.store(oT_ref.at[qb, pl.ds(pl.multiple_of(h * DH - off, 8), VR), :], on, mask=used)

        def pv_dot(h, c, p):
            t, lo = (c * C) // TQ, (c * C) % TQ
            return jnp.dot(vT_ref[t, h, :, lo:lo + C], p, preferred_element_type=F32)

        def ffn_slice(gi):
            r0 = pl.multiple_of(gi * TF, TF)
            xt = x_ref[pl.ds(r0, TF), :]
            hid = jnp.dot(xt, w1_ref[...], preferred_element_type=F32) + b1_ref[...].astype(F32).reshape(1, F)
            r = jnp.maximum(hid, 0.0)
            b = jnp.dot((r * r).astype(BF), w2_ref[...], preferred_element_type=F32) + b2_ref[...].astype(F32).reshape(1, D)
            zz = jnp.sum(xt.astype(F32) * gw_ref[...].astype(F32).reshape(1, D), axis=-1, keepdims=True)
            g = jax.nn.sigmoid(zz)
            c_ref[pl.ds(r0, TF), :] = (1.0 - g) * b
            g_ref[pl.ds(r0, TF), :] = jnp.broadcast_to(g, (TF, 128))

        flat = [(c, 7 - i) for c in range(NC) for i in range(7)]
        ends = [min(len(flat), 7 * (c + 1) + SH) for c in range(NC)]
        bounds = [(st * DH) // NS for st in range(NS + 1)]

        def fast_heads(h0, hh0):
            tmask = lax.broadcasted_iota(I32, (8, 128), 1) >= z_ref[0]
            tasks = [(it, c) for it in range(NQ * NH) for c in range(NC)]
            pieces, accs, chain = {}, {}, {}

            def do_qk(it, c):
                hx, qb = divmod(it, NQ)
                h, hh = h0 + hx, hh0 + hx
                sel = flat[(ends[c - 1] if c else 0):ends[c]]
                kraw = jnp.concatenate(
                    [k_ref[h, tc * 64 + 8 * rg:tc * 64 + 8 * rg + 8, :] for (tc, rg) in sel], axis=0)
                kk = pltpu.bitcast(kraw, BF)[:, :32]
                s = jnp.dot(kk, pltpu.bitcast(qp_ref[qb, h], BF), preferred_element_type=F32)
                for n, key in enumerate(sel):
                    pieces[(it,) + key] = jnp.exp2(s[n * 16:(n + 1) * 16])
                res = [[None] * NL for _ in range(2)]
                for j in range(NL):
                    vac = [None, None]
                    for st in range(NS):
                        for v in range(2):
                            t = None
                            for d in range(bounds[st], bounds[st + 1]):
                                pr = (kb_ref[hh, d, (2 * c + v) * 8:(2 * c + v + 1) * 8, :]
                                      * qb_ref[hh, qb, d, :, j * 128:(j + 1) * 128])
                                t = pr if t is None else t + pr
                            if st == 0 and v in chain:
                                t = jnp.where(tmask, t, chain[v])
                            vac[v] = t if st == 0 else vac[v] + t
                    for v in range(2):
                        res[v][j] = vac[v]
                        chain[v] = vac[v]
                pieces[(it, c, 0)] = jnp.exp2(jnp.concatenate([jnp.concatenate(r, axis=1) for r in res], axis=0))

            def do_pv(it, c):
                hx, qb = divmod(it, NQ)
                h = h0 + hx
                p = jnp.concatenate([pieces.pop((it, c, rg)) for rg in range(8)], axis=0).astype(BF)
                pv = pv_dot(h, c, p)
                accs[it] = pv if c == 0 else pv + accs[it]
                if c == NC - 1:
                    finish(h, hx % 2 if NH % 2 == 0 else h % 2, qb, accs.pop(it))

            for n, tk in enumerate(tasks):
                do_qk(*tk)
                if n >= 1:
                    do_pv(*tasks[n - 1])
            do_pv(*tasks[-1])

        def fast_group(gi, carry):
            with scope("pre"):
                ffn_slice(gi)
                tmask0 = lax.broadcasted_iota(I32, (8, 128), 1) >= z_ref[0]
                for hh in range(GH):
                    for d in range(DH):
                        ln = hh * DH + d
                        kbv = jnp.broadcast_to(kf_ref[gi][:, ln:ln + 1], (R, 128))
                        kb_ref[hh, d] = kbv
                        for qb in range(NQ):
                            qw = q32_ref[qb, pl.ds(pl.multiple_of(gi * (GH * DH) + ln // 8 * 8, 8), 8), :]
                            bq = jnp.broadcast_to(qw[ln % 8:ln % 8 + 1], (8, TQ))
                            for j in range(NL):
                                n = (qb * NL + j) * RG // (NQ * NL)
                                qb_ref[hh, qb, d, :, j * 128:(j + 1) * 128] = jnp.where(
                                    tmask0, bq[:, j * 128:(j + 1) * 128], kbv[n * 8:n * 8 + 8])

            @pl.when(z_ref[0] == 0)
            def _():
                def body(i, c):
                    with scope("fast"):
                        fast_heads(gi * GH + i * NH, i * NH)
                    return c
                lax.fori_loop(0, GH // NH, body, 0)
            return carry

        def slow_item(i, carry):
            h, qb = i // NQ, i % NQ
            qm = pltpu.bitcast(qp_ref[qb, h], BF)
            mx = None
            for c in range(NC):
                kk = pltpu.bitcast(k_ref[h, c * 64:(c + 1) * 64, :], BF)[:, :32]
                s = jnp.dot(kk, qm, preferred_element_type=F32)
                s_ref[c * C:(c + 1) * C, :] = s
                cm = jnp.max(s.reshape(C // 8, 8, TQ), axis=0)
                mx = cm if mx is None else jnp.maximum(mx, cm)
            m = jnp.max(mx, axis=0, keepdims=True)
            acc = None
            for c in range(NC):
                p = jnp.exp2(s_ref[c * C:(c + 1) * C, :] - m).astype(BF)
                pv = pv_dot(h, c, p)
                acc = pv if acc is None else pv + acc
            finish(h, h % 2, qb, acc)
            return carry

        lax.fori_loop(0, NGRP, fast_group, 0)

        @pl.when(z_ref[0] != 0)
        def _():
            lax.fori_loop(0, H * NQ, slow_item, 0)

        def cp_out(e):
            return pltpu.make_async_copy(o_ref.at[pl.ds(e * TE, TE), :], o_hbm.at[0, pl.ds(e * TE, TE), :], sem_out.at[e])

        with scope("epi"):
            for e in range(NE):
                qb, lo = divmod(e * TE, TQ)
                o = oT_ref[qb, :, lo:lo + TE].T.astype(BF)
                a = jnp.dot(o, wo_ref[...], preferred_element_type=F32)
                g = g_ref[e * TE:(e + 1) * TE, :]
                g = jnp.concatenate([g] * (D // 128), axis=1)
                o_ref[e * TE:(e + 1) * TE, :] = (g * a + c_ref[e * TE:(e + 1) * TE, :]).astype(o_ref.dtype)
                cp_out(e).start()
        with scope("outwait"):
            for e in range(NE):
                cp_out(e).wait()

    @jax.jit
    def fn(A_x, A_wqkv, A_wo, B_x, B_w1, B_b1, B_w2, B_b2, gate_w):
        anyspec = pl.BlockSpec(memory_space=pl.ANY)
        return pl.pallas_call(
            kernel,
            in_specs=[anyspec] * 8,
            out_specs=anyspec,
            out_shape=jax.ShapeDtypeStruct((1, S, D), BF),
            scratch_shapes=[
                pltpu.VMEM((S, D), BF),
                pltpu.VMEM((3, D, D), BF),
                pltpu.VMEM((D, D), BF),
                pltpu.VMEM((D, F), BF),
                pltpu.VMEM((F, D), BF),
                pltpu.VMEM((S, D), BF),
                pltpu.VMEM((2 * D, D), BF),
                pltpu.VMEM((S // 2, D), I32),
                pltpu.VMEM((H, S // 2, 128), I32),
                pltpu.VMEM((NQ, H, 16, TQ), I32),
                pltpu.VMEM((NQ, D, TQ), F32),
                pltpu.VMEM((NQ, H, VR, TQ), F32),
                pltpu.VMEM((NQ, D, TQ), F32),
                pltpu.VMEM((S, D), F32),
                pltpu.VMEM((S, 128), F32),
                pltpu.VMEM((NGRP, R, 128), F32),
                pltpu.VMEM((GH, DH, R, 128), F32),
                pltpu.VMEM((GH, NQ, DH, 8, TQ), F32),
                pltpu.VMEM((S, TQ), F32),
                pltpu.VMEM((D, 128), F32),
                pltpu.VMEM((8, D), F32),
                pltpu.VMEM((8, TQ), F32),
                pltpu.VMEM((F,), BF),
                pltpu.VMEM((D,), BF),
                pltpu.VMEM((D,), BF),
                pltpu.SMEM((1,), I32),
                pltpu.SemaphoreType.DMA((NX + 3 + 6,)),
                pltpu.SemaphoreType.DMA((NE,)),
            ],
            compiler_params=pltpu.CompilerParams(vmem_limit_bytes=120 * 1024 * 1024),
            name="gmix",
        )(A_x, A_wqkv, A_wo, B_w1, B_b1, B_w2, B_b2, gate_w)

    return fn


_impl = _make_kernel(TE=128)


@jax.jit
def pallas_gated_mix__softmax_full_mha__dense_activation_squared_relu__prompt_kernel(
    A_x, A_wqkv, A_wo, B_x, B_w1, B_b1, B_w2, B_b2, gate_w):
    return _impl(A_x, A_wqkv, A_wo, B_x, B_w1, B_b1, B_w2, B_b2, gate_w)
```

```python
import contextlib
import math
import jax
import jax.numpy as jnp
from jax import lax
import jax.experimental.pallas as pl
import jax.experimental.pallas.tpu as pltpu

S, D, H, DH, F = 2048, 640, 32, 20, 1536
VR = 24
BF = jnp.bfloat16
F32 = jnp.float32
I32 = jnp.int32


def _make_kernel(TE=128, NH=4, NS=16, SH=1, FORCE=None, TBOUND=60.0, SCOPES=False, PF32=True,
                X0=128, XM=384, NXM=3, EPL=4, GTIE=True, GPOS=2):
    GH = 4
    TQ = 512
    C = 128
    NQ = S // TQ
    NC = S // C
    NE = S // TE
    NL = TQ // 128
    NGRP = H // GH
    TF = S // NGRP
    R = 16 * NC
    RG = R // 8
    QSCALE = (DH ** -0.5) * math.log2(math.e)
    XL = X0 + NXM * XM
    NX = NXM + 2

    def scope(name):
        return jax.named_scope(name) if SCOPES else contextlib.nullcontext()

    def kernel(x_hbm, wqkv_hbm, wo_hbm, w1_hbm, b1_hbm, w2_hbm, b2_hbm, gw_hbm, o_hbm,
               x_ref, wqkv_ref, wo_ref, w1_ref, w2_ref, o_ref,
               wqvT_ref, kn_ref, k_ref, qp_ref, q32_ref, vT_ref, oT_ref, c_ref, g_ref,
               kf_ref, kb_ref, qb_ref, s_ref, qmax_ref, kmax_ref, vmax_ref, b1_ref, b2_ref, gw_ref, z_ref,
               sem_in, sem_out):
        def cp_x(i, lo, n):
            return pltpu.make_async_copy(x_hbm.at[0, pl.ds(lo, n), :], x_ref.at[pl.ds(lo, n), :], sem_in.at[i])

        def cp_xm(i):
            lo = X0 + i * XM
            return cp_x(1 + i, lo if isinstance(i, int) else pl.multiple_of(lo, 128), XM)

        def cp_w(j):
            return pltpu.make_async_copy(wqkv_hbm.at[:, pl.ds(j * D, D)], wqkv_ref.at[j], sem_in.at[NX + j])

        late = [pltpu.make_async_copy(src, dst, sem_in.at[NX + 3 + i])
                for i, (src, dst) in enumerate([(w1_hbm, w1_ref), (w2_hbm, w2_ref), (wo_hbm, wo_ref),
                                                (b1_hbm, b1_ref), (b2_hbm, b2_ref), (gw_hbm, gw_ref)])]
        cp_x0 = cp_x(0, 0, X0)
        cp_xl = cp_x(NX - 1, XL, S - XL)
        cp_x0.start()
        cp_w(1).start()
        for i in range(NXM):
            cp_xm(i).start()
        cp_w(0).start()
        cp_w(2).start()
        cp_xl.start()
        for c in late:
            c.start()
        z_ref[0] = 0

        def lane_window(slabs, start, lane):
            j, o = divmod(start, 128)
            if o == 0:
                return slabs[j]
            a = slabs[j]
            if j + 1 < len(slabs):
                a = jnp.where(lane >= o, a, slabs[j + 1])
            return pltpu.roll(a, 128 - o, 1)

        def kproj(lo, n, first=False):
            def al(v, m):
                return v if isinstance(v, int) else pl.multiple_of(v, m)
            km = None if first else kmax_ref[...]
            lane = lax.broadcasted_iota(I32, (16, 128), 1)
            for i in range(n // 128):
                r = lo + i * 128
                k = jnp.dot(x_ref[pl.ds(al(r, 128), 128), :], wqkv_ref[1], preferred_element_type=F32)
                kn_ref[pl.ds(al(r // 2, 64), 64), :] = pltpu.bitcast(k.astype(BF), I32)
                kr = jnp.max(jnp.abs(k).reshape(16, 8, D), axis=0)
                km = kr if km is None else jnp.maximum(km, kr)
                slabs = [k[0:16, 128 * j:128 * j + 128] for j in range(5)]
                for gi in range(NGRP):
                    kf_ref[gi, pl.ds(al(r // 8, 16), 16), :] = lane_window(slabs, gi * GH * DH, lane)
            kmax_ref[...] = km

        with scope("wait0"):
            cp_x0.wait()
            cp_w(1).wait()
        with scope("kproj"):
            kproj(0, X0, first=True)

            def kbody(i, c):
                cp_xm(i).wait()
                kproj(X0 + i * XM, XM)
                return c
            lax.fori_loop(0, NXM, kbody, 0)
            cp_w(0).wait()
            cp_w(2).wait()
            cp_xl.wait()
            kproj(XL, S - XL)
            wqvT_ref[0:D, :] = wqkv_ref[0].T
            wqvT_ref[D:2 * D, :] = wqkv_ref[2].T
            qmax_ref[...] = jnp.zeros_like(qmax_ref)
            vmax_ref[...] = jnp.zeros_like(vmax_ref)

        def qvproj(t, carry):
            r0 = pl.multiple_of(t * TQ, TQ)
            xt = x_ref[pl.ds(r0, TQ), :]
            qv = lax.dot_general(wqvT_ref[...], xt, (((1,), (1,)), ((), ())), preferred_element_type=F32)
            qf = qv[:D] * QSCALE
            q32_ref[t] = qf
            qa = jnp.abs(qf)
            qm = qmax_ref[...]
            for j in range(NL):
                qm = jnp.maximum(qm, qa[:, 128 * j:128 * j + 128])
            qmax_ref[...] = qm
            v = qv[D:]
            vmax_ref[...] = jnp.maximum(vmax_ref[...], jnp.max(jnp.abs(v).reshape(D // 8, 8, TQ), axis=0))
            row = lax.broadcasted_iota(I32, (VR, TQ), 0)
            zpad = jnp.zeros((32 - VR, TQ), F32)
            for h in range(H):
                off = 4 * (h % 2)
                w = h * DH - off
                used = (row >= off) & (row < off + DH)
                qw = jnp.concatenate([jnp.where(used, qf[w:w + VR], 0.0), zpad], axis=0)
                qp_ref[t, h] = pltpu.bitcast(qw.astype(BF), I32)
                vT_ref[t, h] = jnp.where(used, v[w:w + VR], 1.0)
            rk = pl.multiple_of(t * (TQ // 2), TQ // 2)
            kn = kn_ref[pl.ds(rk, TQ // 2), :]
            slabs = [kn[:, 128 * j:128 * j + 128] for j in range(5)]
            lane = lax.broadcasted_iota(I32, (TQ // 2, 128), 1)
            for h in range(H):
                w = h * DH - 4 * (h % 2)
                j, o = divmod(w, 128)
                sl = slabs[j:j + 2] if o + 32 > 128 else slabs[j:j + 1]
                k_ref[h, pl.ds(rk, TQ // 2), :] = lane_window(sl, o, lane)
            return carry

        with scope("qvproj"):
            lax.fori_loop(0, NQ, qvproj, 0)
        for c in late:
            c.wait()

        def guard(hid):
            qmx = qmax_ref[...]
            if GTIE:
                tie = jnp.concatenate([hid[:, 768:896], hid[:, 896:1024], hid[:D - 2 * TF, 1024:1152]], axis=0)
                qmx = jnp.where(lax.broadcasted_iota(I32, (D, 128), 1) >= z_ref[0], qmx, tie)
            qa = jnp.max(qmx, axis=1, keepdims=True)
            rel = lax.broadcasted_iota(I32, (D, 128), 0) - DH * lax.broadcasted_iota(I32, (D, 128), 1)
            qn2 = jnp.sum(jnp.where((rel >= 0) & (rel < DH), qa * qa, 0.0), axis=0, keepdims=True)
            qn2 = jnp.max(qn2, axis=1, keepdims=True)
            ka = jnp.max(kmax_ref[...], axis=0, keepdims=True)
            rel = lax.broadcasted_iota(I32, (H, D), 1) - DH * lax.broadcasted_iota(I32, (H, D), 0)
            kn2 = jnp.sum(jnp.where((rel >= 0) & (rel < DH), ka * ka, 0.0), axis=1, keepdims=True)
            kn2 = jnp.max(kn2, axis=0, keepdims=True)
            vm = jnp.max(jnp.max(vmax_ref[...], axis=0, keepdims=True), axis=1, keepdims=True)
            safe = (qn2 * kn2 <= TBOUND * TBOUND) & (vm <= 2.0 ** 40) & (vm >= 2.0 ** -40)
            unsafe = jnp.max(jnp.where(safe, 0, 1).astype(I32))
            if FORCE is not None:
                unsafe = jnp.maximum(unsafe, FORCE)
            z_ref[1] = unsafe

        def finish(h, odd, qb, acc):
            off = odd * 4
            if isinstance(odd, int):
                l = acc[0:1] if odd else acc[VR - 1:VR]
            else:
                l = jnp.where(odd == 1, acc[0:1], acc[VR - 1:VR])
            on = acc * (1.0 / l)
            row = lax.broadcasted_iota(I32, (VR, TQ), 0)
            used = (row >= off) & (row < off + DH)
            pltpu.store(oT_ref.at[qb, pl.ds(pl.multiple_of(h * DH - off, 8), VR), :], on, mask=used)

        def ffn_slice(gi):
            r0 = pl.multiple_of(gi * TF, TF)
            xt = x_ref[pl.ds(r0, TF), :]
            hid = jnp.dot(xt, w1_ref[...], preferred_element_type=F32) + b1_ref[...].astype(F32).reshape(1, F)
            r = jnp.maximum(hid, 0.0)
            b = jnp.dot((r * r).astype(BF), w2_ref[...], preferred_element_type=F32) + b2_ref[...].astype(F32).reshape(1, D)
            return hid, b

        def gate(gi, hid, b):
            r0 = pl.multiple_of(gi * TF, TF)
            xg = x_ref[pl.ds(r0, TF), :].astype(F32)
            if GTIE:
                xg = jnp.where(lax.broadcasted_iota(I32, (TF, D), 1) >= z_ref[0], xg, hid[:, :D])
            zz = jnp.sum(xg * gw_ref[...].astype(F32).reshape(1, D), axis=-1, keepdims=True)
            g = jax.nn.sigmoid(zz)
            c_ref[pl.ds(r0, TF), :] = (1.0 - g) * b
            g_ref[pl.ds(r0, TF), :] = jnp.broadcast_to(g, (TF, 128))

        flat = [(c, 7 - i) for c in range(NC) for i in range(7)]
        ends = [min(len(flat), 7 * (c + 1) + SH) for c in range(NC)]
        bounds = [(st * DH) // NS for st in range(NS + 1)]

        def fast_heads(h0, hh0):
            tmask = lax.broadcasted_iota(I32, (2, 8, 128), 2) >= z_ref[0]
            tasks = [(it, c) for it in range(NQ * NH) for c in range(NC)]
            pieces, accs = {}, {}
            chain = [None]

            def do_qk(it, c):
                hx, qb = divmod(it, NQ)
                h, hh = h0 + hx, hh0 + hx
                sel = flat[(ends[c - 1] if c else 0):ends[c]]
                kraw = jnp.concatenate(
                    [k_ref[h, tc * 64 + 8 * rg:tc * 64 + 8 * rg + 8, :] for (tc, rg) in sel], axis=0)
                kk = pltpu.bitcast(kraw, BF)[:, :32]
                e = jnp.exp2(jnp.dot(kk, pltpu.bitcast(qp_ref[qb, h], BF), preferred_element_type=F32))
                for n, key in enumerate(sel):
                    pieces[(it,) + key] = e[n * 16:(n + 1) * 16]
                res = []
                for j in range(NL):
                    kv = kb_ref[hh, :, c * 16:(c + 1) * 16, :].reshape(DH, 2, 8, 128)
                    qv = qb_ref[hh, qb, :, :, j * 128:(j + 1) * 128]
                    pr = kv * qv[:, None]
                    acc = None
                    for st in range(NS):
                        t = pr[bounds[st]]
                        for d in range(bounds[st] + 1, bounds[st + 1]):
                            t = t + pr[d]
                        if st == 0:
                            acc = t if chain[0] is None else jnp.where(tmask, t, chain[0])
                        else:
                            acc = acc + t
                    chain[0] = acc
                    res.append(acc.reshape(16, 128))
                pieces[(it, c, 0)] = jnp.exp2(jnp.concatenate(res, axis=1))

            def do_pv(it, c):
                hx, qb = divmod(it, NQ)
                h = h0 + hx
                p = jnp.concatenate([pieces.pop((it, c, rg)) for rg in range(8)], axis=0)
                if not PF32:
                    p = p.astype(BF)
                t, lo = (c * C) // TQ, (c * C) % TQ
                pv = jnp.dot(vT_ref[t, h, :, lo:lo + C], p, preferred_element_type=F32)
                accs[it] = pv if c == 0 else pv + accs[it]
                if c == NC - 1:
                    finish(h, hx % 2, qb, accs.pop(it))

            for n, tk in enumerate(tasks):
                do_qk(*tk)
                if n >= 1:
                    do_pv(*tasks[n - 1])
            do_pv(*tasks[-1])

        def group(gi, carry):
            with scope("pre"):
                hid, b = ffn_slice(gi)
                tmask0 = lax.broadcasted_iota(I32, (NQ, 8, TQ), 2) >= z_ref[0]
                for hh in range(GH):
                    if hh == GPOS:
                        gate(gi, hid, b)
                        guard(hid)
                    for d in range(DH):
                        ln = hh * DH + d
                        kbv = jnp.broadcast_to(kf_ref[gi][:, ln:ln + 1], (R, 128))
                        kb_ref[hh, d] = kbv
                        qw = q32_ref[:, pl.ds(pl.multiple_of(gi * (GH * DH) + ln // 8 * 8, 8), 8), :]
                        bq = jnp.broadcast_to(qw[:, ln % 8:ln % 8 + 1, :], (NQ, 8, TQ))
                        tie = jnp.stack([jnp.concatenate(
                            [kbv[(qb * NL + j) * 16:(qb * NL + j) * 16 + 8] for j in range(NL)], axis=1)
                            for qb in range(NQ)], axis=0)
                        qb_ref[hh, :, d] = jnp.where(tmask0, bq, tie)

            @pl.when(z_ref[1] == 0)
            def _():
                if NH == GH:
                    with scope("fast"):
                        fast_heads(gi * GH, 0)
                else:
                    def body(i, c):
                        with scope("fast"):
                            fast_heads(gi * GH + i * NH, i * NH)
                        return c
                    lax.fori_loop(0, GH // NH, body, 0)
            return carry

        lax.fori_loop(0, NGRP, group, 0)

        def slow_item(i, carry):
            h, qb = i // NQ, i % NQ

            def pass1(t, mx):
                kk = pltpu.bitcast(k_ref[h, pl.ds(pl.multiple_of(t * (TQ // 2), TQ // 2), TQ // 2), :], BF)[:, :32]
                s = jnp.dot(kk, pltpu.bitcast(qp_ref[qb, h], BF), preferred_element_type=F32)
                s_ref[t] = s
                return jnp.maximum(mx, jnp.max(s.reshape(TQ // 8, 8, TQ), axis=0))
            mx = lax.fori_loop(0, NQ, pass1, jnp.full((8, TQ), -jnp.inf, F32))
            m = jnp.max(mx, axis=0, keepdims=True)

            def pass2(t, acc):
                p = jnp.exp2(s_ref[t] - m).astype(BF)
                return acc + jnp.dot(vT_ref[t, h], p, preferred_element_type=F32)
            acc = lax.fori_loop(0, NQ, pass2, jnp.zeros((VR, TQ), F32))
            finish(h, h % 2, qb, acc)
            return carry

        @pl.when(z_ref[1] != 0)
        def _():
            lax.fori_loop(0, H * NQ, slow_item, 0)

        def cp_out(e):
            r0 = e * TE if isinstance(e, int) else pl.multiple_of(e * TE, TE)
            return pltpu.make_async_copy(o_ref.at[pl.ds(r0, TE), :], o_hbm.at[0, pl.ds(r0, TE), :], sem_out.at[e])

        def epi(i, carry):
            for u in range(NQ // EPL):
                qb = i * (NQ // EPL) + u
                for sub in range(TQ // TE):
                    e = qb * (TQ // TE) + sub
                    r0 = pl.multiple_of(e * TE, TE)
                    o = oT_ref[qb, :, sub * TE:(sub + 1) * TE].T.astype(BF)
                    a = jnp.dot(o, wo_ref[...], preferred_element_type=F32)
                    g = g_ref[pl.ds(r0, TE), :]
                    g = jnp.concatenate([g] * (D // 128), axis=1)
                    o_ref[pl.ds(r0, TE), :] = (g * a + c_ref[pl.ds(r0, TE), :]).astype(o_ref.dtype)
                    cp_out(e).start()
            return carry

        with scope("epi"):
            lax.fori_loop(0, EPL, epi, 0)
        with scope("outwait"):
            for e in range(NE):
                cp_out(e).wait()

    @jax.jit
    def fn(A_x, A_wqkv, A_wo, B_x, B_w1, B_b1, B_w2, B_b2, gate_w):
        anyspec = pl.BlockSpec(memory_space=pl.ANY)
        return pl.pallas_call(
            kernel,
            in_specs=[anyspec] * 8,
            out_specs=anyspec,
            out_shape=jax.ShapeDtypeStruct((1, S, D), BF),
            scratch_shapes=[
                pltpu.VMEM((S, D), BF),
                pltpu.VMEM((3, D, D), BF),
                pltpu.VMEM((D, D), BF),
                pltpu.VMEM((D, F), BF),
                pltpu.VMEM((F, D), BF),
                pltpu.VMEM((S, D), BF),
                pltpu.VMEM((2 * D, D), BF),
                pltpu.VMEM((S // 2, D), I32),
                pltpu.VMEM((H, S // 2, 128), I32),
                pltpu.VMEM((NQ, H, 16, TQ), I32),
                pltpu.VMEM((NQ, D, TQ), F32),
                pltpu.VMEM((NQ, H, VR, TQ), F32),
                pltpu.VMEM((NQ, D, TQ), F32),
                pltpu.VMEM((S, D), F32),
                pltpu.VMEM((S, 128), F32),
                pltpu.VMEM((NGRP, R, 128), F32),
                pltpu.VMEM((GH, DH, R, 128), F32),
                pltpu.VMEM((GH, NQ, DH, 8, TQ), F32),
                pltpu.VMEM((NQ, TQ, TQ), F32),
                pltpu.VMEM((D, 128), F32),
                pltpu.VMEM((8, D), F32),
                pltpu.VMEM((8, TQ), F32),
                pltpu.VMEM((F,), BF),
                pltpu.VMEM((D,), BF),
                pltpu.VMEM((D,), BF),
                pltpu.SMEM((2,), I32),
                pltpu.SemaphoreType.DMA((NX + 3 + 6,)),
                pltpu.SemaphoreType.DMA((NE,)),
            ],
            compiler_params=pltpu.CompilerParams(vmem_limit_bytes=120 * 1024 * 1024),
            name="gmix",
        )(A_x, A_wqkv, A_wo, B_w1, B_b1, B_w2, B_b2, gate_w)

    return fn


_impl = _make_kernel()


@jax.jit
def pallas_gated_mix__softmax_full_mha__dense_activation_squared_relu__prompt_kernel(
    A_x, A_wqkv, A_wo, B_x, B_w1, B_b1, B_w2, B_b2, gate_w):
    return _impl(A_x, A_wqkv, A_wo, B_x, B_w1, B_b1, B_w2, B_b2, gate_w)
```

```python
import math

import jax
import jax.numpy as jnp
from jax import lax
import jax.experimental.pallas as pl
import jax.experimental.pallas.tpu as pltpu

S, D, H, DH, F = 2048, 640, 32, 20, 1536
BF = jnp.bfloat16
F32 = jnp.float32
I32 = jnp.int32

VR = 24
TQ = 512
C = 128
NQ = S // TQ
NC = S // C
NL = TQ // 128
GH = 4
NGRP = H // GH
TF = S // NGRP
R = 16 * NC
TE = 128
NE = S // TE
SFM = 32
X0, XM, NXM = 128, 384, 3
XL = X0 + NXM * XM
NX = NXM + 2
QSCALE = (DH ** -0.5) * math.log2(math.e)
SCORE_BOUND = 60.0
V_HI, V_LO = 2.0 ** 40, 2.0 ** -40

_FLAT = [(c, 7 - i) for c in range(NC) for i in range(7)]
_ENDS = [min(len(_FLAT), 7 * (c + 1) + 1) for c in range(NC)]


def _kernel(x_hbm, wqkv_hbm, wo_hbm, w1_hbm, b1_hbm, w2_hbm, b2_hbm, gw_hbm, o_hbm,
            x_ref, wqkv_ref, wo_ref, w1_ref, w2_ref, o_ref,
            wqvT_ref, kn_ref, k_ref, qp_ref, q32_ref, vT_ref, oT_ref, c_ref, g_ref,
            kf_ref, kb_ref, qb_ref, s_ref, on_ref, qmax_ref, kmax_ref, vmax_ref,
            b1_ref, b2_ref, gw_ref, z_ref, sem_in, sem_out):
    def al(v, m):
        return v if isinstance(v, int) else pl.multiple_of(v, m)

    def true_mask(shape):
        return lax.broadcasted_iota(I32, shape, len(shape) - 1) >= z_ref[0]

    def cp_x(i, lo, n):
        return pltpu.make_async_copy(x_hbm.at[0, pl.ds(lo, n), :], x_ref.at[pl.ds(lo, n), :], sem_in.at[i])

    def cp_xm(i):
        return cp_x(1 + i, al(X0 + i * XM, 128), XM)

    def cp_w(j):
        return pltpu.make_async_copy(wqkv_hbm.at[:, pl.ds(j * D, D)], wqkv_ref.at[j], sem_in.at[NX + j])

    cp_gw = pltpu.make_async_copy(gw_hbm, gw_ref, sem_in.at[0])
    cp_x0 = cp_x(0, 0, X0)
    cp_xl = cp_x(NX - 1, XL, S - XL)
    late = [pltpu.make_async_copy(src, dst, sem_in.at[NX + 3])
            for src, dst in [(w1_hbm, w1_ref), (w2_hbm, w2_ref), (wo_hbm, wo_ref),
                             (b1_hbm, b1_ref), (b2_hbm, b2_ref)]]
    cp_gw.start()
    cp_x0.start()
    cp_w(1).start()
    for i in range(NXM):
        cp_xm(i).start()
    cp_w(0).start()
    cp_w(2).start()
    cp_xl.start()
    for cp in late:
        cp.start()
    z_ref[0] = 0

    def lane_window(slabs, start, lane):
        j, o = divmod(start, 128)
        if o == 0:
            return slabs[j]
        a = slabs[j]
        if j + 1 < len(slabs):
            a = jnp.where(lane >= o, a, slabs[j + 1])
        return pltpu.roll(a, 128 - o, 1)

    def kproj(lo, n, first=False):
        km = None if first else kmax_ref[...]
        gw = gw_ref[...].astype(F32).reshape(1, D)
        lane = lax.broadcasted_iota(I32, (16, 128), 1)
        k = None
        for i in range(n // 128):
            r = lo + i * 128
            xt = x_ref[pl.ds(al(r, 128), 128), :]
            xg = xt.astype(F32)
            if k is not None:
                xg = jnp.where(true_mask((128, D)), xg, k)
            zz = jnp.sum(xg * gw, axis=-1, keepdims=True)
            g_ref[pl.ds(al(r, 128), 128), :] = jnp.broadcast_to(jax.nn.sigmoid(zz), (128, 128))
            k = jnp.dot(xt, wqkv_ref[1], preferred_element_type=F32)
            kn_ref[pl.ds(al(r // 2, 64), 64), :] = pltpu.bitcast(k.astype(BF), I32)
            kr = jnp.max(jnp.abs(k).reshape(16, 8, D), axis=0)
            km = kr if km is None else jnp.maximum(km, kr)
            slabs = [k[0:16, 128 * j:128 * j + 128] for j in range(D // 128)]
            for gi in range(NGRP):
                kf_ref[gi, pl.ds(al(r // 8, 16), 16), :] = lane_window(slabs, gi * GH * DH, lane)
        kmax_ref[...] = km

    cp_gw.wait()
    cp_x0.wait()
    cp_w(1).wait()
    kproj(0, X0, first=True)

    def kproj_mid(i, carry):
        cp_xm(i).wait()
        kproj(X0 + i * XM, XM)
        return carry

    lax.fori_loop(0, NXM, kproj_mid, 0)
    cp_w(0).wait()
    cp_w(2).wait()
    cp_xl.wait()
    wqvT_ref[0:D, :] = wqkv_ref[0].T
    wqvT_ref[D:2 * D, :] = wqkv_ref[2].T
    kproj(XL, S - XL)
    qmax_ref[...] = jnp.zeros_like(qmax_ref)
    vmax_ref[...] = jnp.zeros_like(vmax_ref)

    def qvproj(t, carry):
        xt = x_ref[pl.ds(pl.multiple_of(t * TQ, TQ), TQ), :]
        qv = lax.dot_general(wqvT_ref[...], xt, (((1,), (1,)), ((), ())), preferred_element_type=F32)
        qf = qv[:D] * QSCALE
        q32_ref[t] = qf
        v = qv[D:]
        vmax_ref[...] = jnp.maximum(vmax_ref[...], jnp.max(jnp.abs(v).reshape(D // 8, 8, TQ), axis=0))
        row = lax.broadcasted_iota(I32, (VR, TQ), 0)
        zpad = jnp.zeros((32 - VR, TQ), F32)
        qm = qmax_ref[...]
        for h in range(H):
            off = 4 * (h % 2)
            w = h * DH - off
            used = (row >= off) & (row < off + DH)
            qw = jnp.where(used, qf[w:w + VR], 0.0)
            qm = jnp.maximum(qm, jnp.sum((qw * qw).reshape(VR // 8, 8, TQ), axis=0))
            qp_ref[t, h] = pltpu.bitcast(jnp.concatenate([qw, zpad], axis=0).astype(BF), I32)
            vT_ref[t, h] = jnp.where(used, v[w:w + VR], 1.0)
        qmax_ref[...] = qm
        rk = pl.multiple_of(t * (TQ // 2), TQ // 2)
        kn = kn_ref[pl.ds(rk, TQ // 2), :]
        slabs = [kn[:, 128 * j:128 * j + 128] for j in range(D // 128)]
        lane = lax.broadcasted_iota(I32, (TQ // 2, 128), 1)
        for h in range(H):
            j, o = divmod(h * DH - 4 * (h % 2), 128)
            sl = slabs[j:j + 2] if o + 32 > 128 else slabs[j:j + 1]
            k_ref[h, pl.ds(rk, TQ // 2), :] = lane_window(sl, o, lane)
        nr = R // NQ
        rr = pl.multiple_of(t * nr, nr)
        for ln in range(GH * DH):
            hh, d = divmod(ln, DH)
            kb_ref[hh, d, pl.ds(rr, nr), :] = jnp.broadcast_to(kf_ref[0, pl.ds(rr, nr), ln:ln + 1], (nr, 128))
            qb_ref[hh, t, d, :, 0:TQ] = jnp.broadcast_to(qf[ln:ln + 1], (8, TQ))
        return carry

    lax.fori_loop(0, NQ, qvproj, 0)
    for cp in late:
        cp.wait()

    qn2 = jnp.sum(jnp.max(qmax_ref[...], axis=1, keepdims=True), axis=0, keepdims=True)
    ka = jnp.max(kmax_ref[...], axis=0, keepdims=True)
    rel = lax.broadcasted_iota(I32, (H, D), 1) - DH * lax.broadcasted_iota(I32, (H, D), 0)
    kn2 = jnp.sum(jnp.where((rel >= 0) & (rel < DH), ka * ka, 0.0), axis=1, keepdims=True)
    kn2 = jnp.max(kn2, axis=0, keepdims=True)
    vm = jnp.max(jnp.max(vmax_ref[...], axis=0, keepdims=True), axis=1, keepdims=True)
    safe = (qn2 * kn2 <= SCORE_BOUND * SCORE_BOUND) & (vm <= V_HI) & (vm >= V_LO)
    z_ref[1] = jnp.max(jnp.where(safe, 0, 1).astype(I32))

    def finish(h, odd, qb, acc):
        off = odd * 4
        if isinstance(odd, int):
            l = acc[0:1] if odd else acc[VR - 1:VR]
        else:
            l = jnp.where(odd == 1, acc[0:1], acc[VR - 1:VR])
        row = lax.broadcasted_iota(I32, (VR, TQ), 0)
        used = (row >= off) & (row < off + DH)
        pltpu.store(oT_ref.at[qb, pl.ds(pl.multiple_of(h * DH - off, 8), VR), :], acc * (1.0 / l), mask=used)

    def ffn_rows(i, n, mid=None):
        r0 = pl.multiple_of(i * n, n)
        hid = jnp.dot(x_ref[pl.ds(r0, n), :], w1_ref[...], preferred_element_type=F32)
        hid = hid + b1_ref[...].astype(F32).reshape(1, F)
        if mid is not None:
            mid()
        r = jnp.maximum(hid, 0.0)
        b = jnp.dot((r * r).astype(BF), w2_ref[...], preferred_element_type=F32)
        b = b + b2_ref[...].astype(F32).reshape(1, D)
        g = g_ref[pl.ds(r0, n), :]
        c_ref[pl.ds(r0, n), :] = (1.0 - jnp.concatenate([g] * (D // 128), axis=1)) * b

    def fast_group(gi, carry):
        h0 = gi * GH
        link = true_mask((1, 2, 8, 128))
        tasks = [(it, c) for it in range(GH * NQ) for c in range(NC)]
        pieces, accs = {}, {}
        chain = [None]

        def scores(it, c):
            hh, qb = divmod(it, NQ)
            h = h0 + hh
            sel = _FLAT[(_ENDS[c - 1] if c else 0):_ENDS[c]]
            kraw = jnp.concatenate(
                [k_ref[h, tc * 64 + 8 * rg:tc * 64 + 8 * rg + 8, :] for (tc, rg) in sel], axis=0)
            kk = pltpu.bitcast(kraw, BF)[:, :32]
            e = jnp.exp2(jnp.dot(kk, pltpu.bitcast(qp_ref[qb, h], BF), preferred_element_type=F32))
            for n, key in enumerate(sel):
                pieces[(it,) + key] = e[n * 16:(n + 1) * 16]
            res = []
            for j in range(NL):
                kv = kb_ref[hh, :, c * 16:(c + 1) * 16, :].reshape(DH, 2, 8, 128)
                qv = qb_ref[hh, qb, :, :, j * 128:(j + 1) * 128]
                p5 = (kv * qv[:, None]).reshape(4, 5, 2, 8, 128)
                terms = jnp.concatenate([p5[:, 0:3], p5[:, 3:4] + p5[:, 4:5]], axis=1).reshape(16, 2, 8, 128)
                if chain[0] is not None:
                    terms = jnp.concatenate([jnp.where(link, terms[0:1], chain[0][None]), terms[1:]], axis=0)
                chain[0] = jnp.sum(terms, axis=0)
                res.append(chain[0].reshape(16, 128))
            pieces[(it, c, 0)] = jnp.exp2(jnp.concatenate(res, axis=1))

        def pv(it, c):
            hh, qb = divmod(it, NQ)
            p = jnp.concatenate([pieces.pop((it, c, rg)) for rg in range(8)], axis=0)
            t, lo = divmod(c * C, TQ)
            o = jnp.dot(vT_ref[t, h0 + hh, :, lo:lo + C], p, preferred_element_type=F32)
            accs[it] = o if c == 0 else o + accs[it]
            if c == NC - 1:
                finish(h0 + hh, hh % 2, qb, accs.pop(it))

        for n, task in enumerate(tasks):
            scores(*task)
            if n >= 1:
                pv(*tasks[n - 1])
        ffn_rows(gi, TF, mid=lambda: pv(*tasks[-1]))

        gn = jnp.minimum(gi + 1, NGRP - 1)
        pace = true_mask((NQ, 8, TQ))
        for ln in range(GH * DH):
            hh, d = divmod(ln, DH)
            kbv = jnp.broadcast_to(kf_ref[gn][:, ln:ln + 1], (R, 128))
            kb_ref[hh, d, 0:R, :] = kbv
            qw = q32_ref[:, pl.ds(pl.multiple_of(gn * (GH * DH) + ln // 8 * 8, 8), 8), :]
            bq = jnp.broadcast_to(qw[:, ln % 8:ln % 8 + 1, :], (NQ, 8, TQ))
            tie = jnp.stack([jnp.concatenate(
                [kbv[(qb * NL + j) * 16:(qb * NL + j) * 16 + 8] for j in range(NL)], axis=1)
                for qb in range(NQ)], axis=0)
            qb_ref[hh, :, d, :, 0:TQ] = jnp.where(pace, bq, tie)
        return carry

    @pl.when(z_ref[1] == 0)
    def _():
        lax.fori_loop(0, NGRP, fast_group, 0)

    def slow_ffn(i, carry):
        ffn_rows(i, SFM)
        return carry

    def slow_item(i, carry):
        h, qb = i // NQ, i % NQ

        def pass1(t, mx):
            kk = pltpu.bitcast(k_ref[h, pl.ds(pl.multiple_of(t * (TQ // 2), TQ // 2), TQ // 2), :], BF)[:, :32]
            s = jnp.dot(kk, pltpu.bitcast(qp_ref[qb, h], BF), preferred_element_type=F32)
            s_ref[t] = s
            return jnp.maximum(mx, jnp.max(s.reshape(TQ // 8, 8, TQ), axis=0))

        mx = lax.fori_loop(0, NQ, pass1, jnp.full((8, TQ), -jnp.inf, F32))
        m = jnp.max(mx, axis=0, keepdims=True)

        def pass2(t, acc):
            p = jnp.exp2(s_ref[t] - m).astype(BF)
            return acc + jnp.dot(vT_ref[t, h], p, preferred_element_type=F32)

        finish(h, h % 2, qb, lax.fori_loop(0, NQ, pass2, jnp.zeros((VR, TQ), F32)))
        return carry

    @pl.when(z_ref[1] != 0)
    def _():
        lax.fori_loop(0, S // SFM, slow_ffn, 0)
        lax.fori_loop(0, H * NQ, slow_item, 0)

    def cp_out(e):
        r0 = al(e * TE, TE)
        return pltpu.make_async_copy(o_ref.at[pl.ds(r0, TE), :], o_hbm.at[0, pl.ds(r0, TE), :], sem_out.at[0])

    def o_chunk(qb, sub):
        return oT_ref[qb, :, sub * TE:(sub + 1) * TE].T.astype(BF)

    def epilogue(qb, carry):
        for sub in range(TQ // TE):
            e = qb * (TQ // TE) + sub
            r0 = pl.multiple_of(e * TE, TE)
            o = pltpu.bitcast(on_ref[...], BF) if sub == 0 else o_chunk(qb, sub)
            a = jnp.dot(o, wo_ref[...], preferred_element_type=F32)
            g = jnp.concatenate([g_ref[pl.ds(r0, TE), :]] * (D // 128), axis=1)
            o_ref[pl.ds(r0, TE), :] = (g * a + c_ref[pl.ds(r0, TE), :]).astype(o_ref.dtype)
            cp_out(e).start()
        on_ref[...] = pltpu.bitcast(o_chunk(jnp.minimum(qb + 1, NQ - 1), 0), I32)
        return carry

    on_ref[...] = pltpu.bitcast(o_chunk(0, 0), I32)
    lax.fori_loop(0, NQ, epilogue, 0)
    for e in range(NE):
        cp_out(e).wait()


@jax.jit
def pallas_gated_mix__softmax_full_mha__dense_activation_squared_relu__prompt_kernel(
    A_x: jax.Array,
    A_wqkv: jax.Array,
    A_wo: jax.Array,
    B_x: jax.Array,
    B_w1: jax.Array,
    B_b1: jax.Array,
    B_w2: jax.Array,
    B_b2: jax.Array,
    gate_w: jax.Array,
):
    del B_x
    hbm = pl.BlockSpec(memory_space=pl.ANY)
    return pl.pallas_call(
        _kernel,
        in_specs=[hbm] * 8,
        out_specs=hbm,
        out_shape=jax.ShapeDtypeStruct((1, S, D), BF),
        scratch_shapes=[
            pltpu.VMEM((S, D), BF),
            pltpu.VMEM((3, D, D), BF),
            pltpu.VMEM((D, D), BF),
            pltpu.VMEM((D, F), BF),
            pltpu.VMEM((F, D), BF),
            pltpu.VMEM((S, D), BF),
            pltpu.VMEM((2 * D, D), BF),
            pltpu.VMEM((S // 2, D), I32),
            pltpu.VMEM((H, S // 2, 128), I32),
            pltpu.VMEM((NQ, H, 16, TQ), I32),
            pltpu.VMEM((NQ, D, TQ), F32),
            pltpu.VMEM((NQ, H, VR, TQ), F32),
            pltpu.VMEM((NQ, D, TQ), F32),
            pltpu.VMEM((S, D), F32),
            pltpu.VMEM((S, 128), F32),
            pltpu.VMEM((NGRP, R, 128), F32),
            pltpu.VMEM((GH, DH, R + 8, 128), F32),
            pltpu.VMEM((GH, NQ, DH, 8, TQ + 128), F32),
            pltpu.VMEM((NQ, TQ, TQ), F32),
            pltpu.VMEM((TE // 2, D), I32),
            pltpu.VMEM((8, TQ), F32),
            pltpu.VMEM((8, D), F32),
            pltpu.VMEM((8, TQ), F32),
            pltpu.VMEM((F,), BF),
            pltpu.VMEM((D,), BF),
            pltpu.VMEM((D,), BF),
            pltpu.SMEM((2,), I32),
            pltpu.SemaphoreType.DMA((NX + 4,)),
            pltpu.SemaphoreType.DMA((1,)),
        ],
        compiler_params=pltpu.CompilerParams(vmem_limit_bytes=120 * 1024 * 1024),
        name="gated_mix",
    )(A_x, A_wqkv, A_wo, B_w1, B_b1, B_w2, B_b2, gate_w)
```

```python
import math

import jax
import jax.numpy as jnp
from jax import lax
import jax.experimental.pallas as pl
import jax.experimental.pallas.tpu as pltpu

S, D, H, DH, F = 2048, 640, 32, 20, 1536
BF = jnp.bfloat16
F32 = jnp.float32
I32 = jnp.int32

VR = 24
TQ = 512
C = 128
NQ = S // TQ
NC = S // C
NL = TQ // 128
GH = 4
NGRP = H // GH
TF = S // NGRP
R = 16 * NC
TE = 128
NE = S // TE
SFM = 32
X0, XM, NXM = 128, 384, 3
XL = X0 + NXM * XM
NX = NXM + 2
QSCALE = (DH ** -0.5) * math.log2(math.e)
SCORE_BOUND = 60.0
V_HI, V_LO = 2.0 ** 40, 2.0 ** -40
assert NQ == 4 and NL == 4


def _kernel(x_hbm, wqkv_hbm, wo_hbm, w1_hbm, b1_hbm, w2_hbm, b2_hbm, gw_hbm, o_hbm,
            x_ref, wqkv_ref, wo_ref, w1_ref, w2_ref, o_ref,
            wqvT_ref, kn_ref, k_ref, qp_ref, q32_ref, vT_ref, oT_ref, c_ref, g_ref,
            kf_ref, kb_ref, qb_ref, s_ref, on_ref, qmax_ref, kmax_ref, vmax_ref,
            b1_ref, b2_ref, gw_ref, z_ref, sem_in, sem_out):
    def al(v, m):
        return v if isinstance(v, int) else pl.multiple_of(v, m)

    def true_mask(shape):
        return lax.broadcasted_iota(I32, shape, len(shape) - 1) >= z_ref[0]

    def cp_x(i, lo, n):
        return pltpu.make_async_copy(x_hbm.at[0, pl.ds(lo, n), :], x_ref.at[pl.ds(lo, n), :], sem_in.at[i])

    def cp_xm(i):
        return cp_x(1 + i, al(X0 + i * XM, 128), XM)

    def cp_w(j):
        return pltpu.make_async_copy(wqkv_hbm.at[:, pl.ds(j * D, D)], wqkv_ref.at[j], sem_in.at[NX + j])

    cp_gw = pltpu.make_async_copy(gw_hbm, gw_ref, sem_in.at[0])
    cp_x0 = cp_x(0, 0, X0)
    cp_xl = cp_x(NX - 1, XL, S - XL)
    late = [pltpu.make_async_copy(src, dst, sem_in.at[NX + 3])
            for src, dst in [(w1_hbm, w1_ref), (w2_hbm, w2_ref), (wo_hbm, wo_ref),
                             (b1_hbm, b1_ref), (b2_hbm, b2_ref)]]
    cp_gw.start()
    cp_x0.start()
    cp_w(1).start()
    for i in range(NXM):
        cp_xm(i).start()
    cp_w(0).start()
    cp_w(2).start()
    cp_xl.start()
    for cp in late:
        cp.start()
    z_ref[0] = 0

    def lane_window(slabs, start, lane):
        j, o = divmod(start, 128)
        if o == 0:
            return slabs[j]
        a = slabs[j]
        if j + 1 < len(slabs):
            a = jnp.where(lane >= o, a, slabs[j + 1])
        return pltpu.roll(a, 128 - o, 1)

    def kproj(lo, n, first=False):
        km = None if first else kmax_ref[...]
        gw = gw_ref[...].astype(F32).reshape(1, D)
        lane = lax.broadcasted_iota(I32, (16, 128), 1)
        k = None
        for i in range(n // 128):
            r = lo + i * 128
            xt = x_ref[pl.ds(al(r, 128), 128), :]
            xg = xt.astype(F32)
            if k is not None:
                xg = jnp.where(true_mask((128, D)), xg, k)
            zz = jnp.sum(xg * gw, axis=-1, keepdims=True)
            g_ref[pl.ds(al(r, 128), 128), :] = jnp.broadcast_to(jax.nn.sigmoid(zz), (128, 128))
            k = jnp.dot(xt, wqkv_ref[1], preferred_element_type=F32)
            kn_ref[pl.ds(al(r >> 1, 64), 64), :] = pltpu.bitcast(k.astype(BF), I32)
            kr = jnp.max(jnp.abs(k).reshape(16, 8, D), axis=0)
            km = kr if km is None else jnp.maximum(km, kr)
            slabs = [k[0:16, 128 * j:128 * j + 128] for j in range(D // 128)]
            rows = pl.ds(al(r >> 3, 16), 16)
            for gi in range(NGRP):
                kf_ref[gi, rows, :] = lane_window(slabs, gi * GH * DH, lane)
        kmax_ref[...] = km

    cp_gw.wait()
    cp_x0.wait()
    cp_w(1).wait()
    kproj(0, X0, first=True)

    def kproj_mid(i, carry):
        cp_xm(i).wait()
        kproj(X0 + i * XM, XM)
        return carry

    lax.fori_loop(0, NXM, kproj_mid, 0)
    cp_w(0).wait()
    cp_w(2).wait()
    cp_xl.wait()
    wqvT_ref[0:D, :] = wqkv_ref[0].T
    wqvT_ref[D:2 * D, :] = wqkv_ref[2].T
    kproj(XL, S - XL)
    qmax_ref[...] = jnp.zeros_like(qmax_ref)
    vmax_ref[...] = jnp.zeros_like(vmax_ref)

    def qvproj(t, carry):
        xt = x_ref[pl.ds(pl.multiple_of(t * TQ, TQ), TQ), :]
        qv = lax.dot_general(wqvT_ref[...], xt, (((1,), (1,)), ((), ())), preferred_element_type=F32)
        qf = qv[:D] * QSCALE
        q32_ref[t] = qf
        v = qv[D:]
        vmax_ref[...] = jnp.maximum(vmax_ref[...], jnp.max(jnp.abs(v).reshape(D // 8, 8, TQ), axis=0))
        row = lax.broadcasted_iota(I32, (VR, TQ), 0)
        zpad = jnp.zeros((32 - VR, TQ), F32)
        qm = qmax_ref[...]
        for h in range(H):
            off = 4 * (h % 2)
            w = h * DH - off
            used = (row >= off) & (row < off + DH)
            qw = jnp.where(used, qf[w:w + VR], 0.0)
            qm = jnp.maximum(qm, jnp.sum((qw * qw).reshape(VR // 8, 8, TQ), axis=0))
            qp_ref[t, h] = pltpu.bitcast(jnp.concatenate([qw, zpad], axis=0).astype(BF), I32)
            vT_ref[t, h] = jnp.where(used, v[w:w + VR], 1.0)
        qmax_ref[...] = qm
        rk = pl.multiple_of(t * (TQ // 2), TQ // 2)
        kn = kn_ref[pl.ds(rk, TQ // 2), :]
        slabs = [kn[:, 128 * j:128 * j + 128] for j in range(D // 128)]
        lane = lax.broadcasted_iota(I32, (TQ // 2, 128), 1)
        for h in range(H):
            j, o = divmod(h * DH - 4 * (h % 2), 128)
            sl = slabs[j:j + 2] if o + 32 > 128 else slabs[j:j + 1]
            k_ref[h, pl.ds(rk, TQ // 2), :] = lane_window(sl, o, lane)
        nr = R // NQ
        rr = pl.multiple_of(t * nr, nr)
        for ln in range(GH * DH):
            hh, d = divmod(ln, DH)
            kb_ref[hh, d, pl.ds(rr, nr), :] = jnp.broadcast_to(kf_ref[0, pl.ds(rr, nr), ln:ln + 1], (nr, 128))
            bq = jnp.broadcast_to(qf[ln:ln + 1], (8, TQ))
            for j in range(NL):
                qb_ref[hh, t, d, j] = bq[:, 128 * j:128 * j + 128]
        return carry

    lax.fori_loop(0, NQ, qvproj, 0)
    for cp in late:
        cp.wait()

    qn2 = jnp.sum(jnp.max(qmax_ref[...], axis=1, keepdims=True), axis=0, keepdims=True)
    ka = jnp.max(kmax_ref[...], axis=0, keepdims=True)
    rel = lax.broadcasted_iota(I32, (H, D), 1) - DH * lax.broadcasted_iota(I32, (H, D), 0)
    kn2 = jnp.sum(jnp.where((rel >= 0) & (rel < DH), ka * ka, 0.0), axis=1, keepdims=True)
    kn2 = jnp.max(kn2, axis=0, keepdims=True)
    vm = jnp.max(jnp.max(vmax_ref[...], axis=0, keepdims=True), axis=1, keepdims=True)
    safe = (qn2 * kn2 <= SCORE_BOUND * SCORE_BOUND) & (vm <= V_HI) & (vm >= V_LO)
    unsafe = jnp.max(jnp.where(safe, 0, 1).astype(I32))

    def finish(h, odd, qb, acc):
        off = odd * 4
        l = jnp.where(odd == 1, acc[0:1], acc[VR - 1:VR])
        row = lax.broadcasted_iota(I32, (VR, TQ), 0)
        used = (row >= off) & (row < off + DH)
        pltpu.store(oT_ref.at[qb, pl.ds(pl.multiple_of(h * DH - off, 8), VR), :], acc * (1.0 / l), mask=used)

    def ffn_rows(i, n, mid=None):
        r0 = pl.multiple_of(i * n, n)
        hid = jnp.dot(x_ref[pl.ds(r0, n), :], w1_ref[...], preferred_element_type=F32)
        hid = hid + b1_ref[...].astype(F32).reshape(1, F)
        if mid is not None:
            mid()
        r = jnp.maximum(hid, 0.0)
        b = jnp.dot((r * r).astype(BF), w2_ref[...], preferred_element_type=F32)
        b = b + b2_ref[...].astype(F32).reshape(1, D)
        g = g_ref[pl.ds(r0, n), :]
        c_ref[pl.ds(r0, n), :] = (1.0 - jnp.concatenate([g] * (D // 128), axis=1)) * b

    def fast_group(gi, carry):
        h0 = gi * GH
        link = true_mask((1, 1, 16, 128))

        def ids(it):
            hh, qb = it >> 2, it & 3
            return hh, qb, h0 + hh

        def scores(idx, c, top, ahead, chain):
            hh, qb, h = idx
            kt = k_ref[h, pl.ds(al(c * 64, 64), 128 if ahead else 64), :]
            groups = list(range(top, 0, -1)) + ([15] if ahead else [])
            kk = pltpu.bitcast(jnp.concatenate([kt[8 * rg:8 * rg + 8] for rg in groups], axis=0), BF)[:, :32]
            e = jnp.exp2(jnp.dot(kk, pltpu.bitcast(qp_ref[qb, h], BF), preferred_element_type=F32))
            pieces = {rg: e[n * 16:(n + 1) * 16] for n, rg in enumerate(groups)}
            kv = kb_ref[hh, :, pl.ds(al(c * 16, 16), 16), :].reshape(4, 5, 1, 2, 8, 128)
            p5 = kv * qb_ref[hh, qb, :, 0:NL].reshape(4, 5, NL, 1, 8, 128)
            terms = jnp.concatenate([p5[:, 0:3], p5[:, 3:4] + p5[:, 4:5]], axis=1).reshape(16, NL, 16, 128)
            res = []
            for j in range(NL):
                head = terms[0:1, j:j + 1]
                if chain is not None:
                    head = jnp.where(link, head, chain)
                chain = jnp.sum(jnp.concatenate([head, terms[1:, j:j + 1]], axis=0), axis=0, keepdims=True)
                res.append(chain.reshape(16, 128))
            pieces[0] = jnp.exp2(jnp.concatenate(res, axis=1))
            return pieces, chain

        def tile(pieces):
            return jnp.concatenate([pieces[rg] for rg in range(8)], axis=0)

        def pv(idx, c, p):
            vw = vT_ref[c >> 2, idx[2], :, pl.ds(al((c & 3) * C, C), C)]
            return jnp.dot(vw, p, preferred_element_type=F32)

        def close(it, p, acc):
            idx = ids(it)
            finish(idx[2], idx[0] & 1, idx[1], pv(idx, NC - 1, p) + acc)

        def item(it, state):
            chain, p_last, acc_last = state
            idx = ids(it)
            pieces, chain = scores(idx, 0, 7, True, chain)
            if p_last is not None:
                close(it - 1, p_last, acc_last)
            p, ahead = tile(pieces), pieces[15]
            pieces, chain = scores(idx, 1, 6, True, chain)
            acc = pv(idx, 0, p)
            p, ahead = tile({**pieces, 7: ahead}), pieces[15]

            def mid(c, st):
                chain, p, ahead, acc = st
                pieces, chain = scores(idx, c, 6, True, chain)
                return chain, tile({**pieces, 7: ahead}), pieces[15], pv(idx, c - 1, p) + acc

            chain, p, ahead, acc = lax.fori_loop(2, NC - 1, mid, (chain, p, ahead, acc), unroll=True)
            pieces, chain = scores(idx, NC - 1, 6, False, chain)
            acc = pv(idx, NC - 2, p) + acc
            return chain, tile({**pieces, 7: ahead}), acc

        state = item(0, (None, None, None))
        _, p_last, acc_last = lax.fori_loop(1, GH * NQ, item, state, unroll=True)
        ffn_rows(gi, TF, mid=lambda: close(GH * NQ - 1, p_last, acc_last))

        gn = jnp.minimum(gi + 1, NGRP - 1)
        pace = true_mask((NQ, NL, 8, 128))
        for ln in range(GH * DH):
            hh, d = divmod(ln, DH)
            kbv = jnp.broadcast_to(kf_ref[gn][:, ln:ln + 1], (R, 128))
            kb_ref[hh, d, 0:R, :] = kbv
            qw = q32_ref[:, pl.ds(pl.multiple_of(gn * (GH * DH) + ln // 8 * 8, 8), 8), :]
            bq = jnp.broadcast_to(qw[:, ln % 8:ln % 8 + 1, :], (NQ, 8, TQ))
            bq = jnp.stack([bq[:, :, 128 * j:128 * j + 128] for j in range(NL)], axis=1)
            tie = kbv.reshape(NQ, NL, 16, 128)[:, :, 0:8]
            qb_ref[hh, :, d, 0:NL] = jnp.where(pace, bq, tie)
        return carry

    def fast_path():
        lax.fori_loop(0, NGRP, fast_group, 0)

    def slow_ffn(i, carry):
        ffn_rows(i, SFM)
        return carry

    def slow_item(i, carry):
        h, qb = i >> 2, i & 3

        def pass1(t, mx):
            kk = pltpu.bitcast(k_ref[h, pl.ds(pl.multiple_of(t * (TQ // 2), TQ // 2), TQ // 2), :], BF)[:, :32]
            s = jnp.dot(kk, pltpu.bitcast(qp_ref[qb, h], BF), preferred_element_type=F32)
            s_ref[t] = s
            return jnp.maximum(mx, jnp.max(s.reshape(TQ // 8, 8, TQ), axis=0))

        mx = lax.fori_loop(0, NQ, pass1, jnp.full((8, TQ), -jnp.inf, F32))
        m = jnp.max(mx, axis=0, keepdims=True)

        def pass2(t, acc):
            p = jnp.exp2(s_ref[t] - m).astype(BF)
            return acc + jnp.dot(vT_ref[t, h], p, preferred_element_type=F32)

        finish(h, h & 1, qb, lax.fori_loop(0, NQ, pass2, jnp.zeros((VR, TQ), F32)))
        return carry

    def slow_path():
        lax.fori_loop(0, S // SFM, slow_ffn, 0)
        lax.fori_loop(0, H * NQ, slow_item, 0)

    lax.cond(unsafe == 0, fast_path, slow_path)

    def cp_out(e):
        r0 = al(e * TE, TE)
        return pltpu.make_async_copy(o_ref.at[pl.ds(r0, TE), :], o_hbm.at[0, pl.ds(r0, TE), :], sem_out.at[0])

    def o_chunk(qb, sub):
        return oT_ref[qb, :, sub * TE:(sub + 1) * TE].T.astype(BF)

    def epilogue(qb, carry):
        for sub in range(TQ // TE):
            e = qb * (TQ // TE) + sub
            r0 = pl.multiple_of(e * TE, TE)
            o = pltpu.bitcast(on_ref[...], BF) if sub == 0 else o_chunk(qb, sub)
            a = jnp.dot(o, wo_ref[...], preferred_element_type=F32)
            g = jnp.concatenate([g_ref[pl.ds(r0, TE), :]] * (D // 128), axis=1)
            o_ref[pl.ds(r0, TE), :] = (g * a + c_ref[pl.ds(r0, TE), :]).astype(o_ref.dtype)
            cp_out(e).start()
        on_ref[...] = pltpu.bitcast(o_chunk(jnp.minimum(qb + 1, NQ - 1), 0), I32)
        return carry

    on_ref[...] = pltpu.bitcast(o_chunk(0, 0), I32)
    lax.fori_loop(0, NQ, epilogue, 0)
    for e in range(NE):
        cp_out(e).wait()


@jax.jit
def pallas_gated_mix__softmax_full_mha__dense_activation_squared_relu__prompt_kernel(
    A_x: jax.Array,
    A_wqkv: jax.Array,
    A_wo: jax.Array,
    B_x: jax.Array,
    B_w1: jax.Array,
    B_b1: jax.Array,
    B_w2: jax.Array,
    B_b2: jax.Array,
    gate_w: jax.Array,
):
    del B_x
    hbm = pl.BlockSpec(memory_space=pl.ANY)
    return pl.pallas_call(
        _kernel,
        in_specs=[hbm] * 8,
        out_specs=hbm,
        out_shape=jax.ShapeDtypeStruct((1, S, D), BF),
        scratch_shapes=[
            pltpu.VMEM((S, D), BF),
            pltpu.VMEM((3, D, D), BF),
            pltpu.VMEM((D, D), BF),
            pltpu.VMEM((D, F), BF),
            pltpu.VMEM((F, D), BF),
            pltpu.VMEM((S, D), BF),
            pltpu.VMEM((2 * D, D), BF),
            pltpu.VMEM((S // 2, D), I32),
            pltpu.VMEM((H, S // 2, 128), I32),
            pltpu.VMEM((NQ, H, 16, TQ), I32),
            pltpu.VMEM((NQ, D, TQ), F32),
            pltpu.VMEM((NQ, H, VR, TQ), F32),
            pltpu.VMEM((NQ, D, TQ), F32),
            pltpu.VMEM((S, D), F32),
            pltpu.VMEM((S, 128), F32),
            pltpu.VMEM((NGRP, R, 128), F32),
            pltpu.VMEM((GH, DH, R + 8, 128), F32),
            pltpu.VMEM((GH, NQ, DH, NL + 1, 8, 128), F32),
            pltpu.VMEM((NQ, TQ, TQ), F32),
            pltpu.VMEM((TE // 2, D), I32),
            pltpu.VMEM((8, TQ), F32),
            pltpu.VMEM((8, D), F32),
            pltpu.VMEM((8, TQ), F32),
            pltpu.VMEM((F,), BF),
            pltpu.VMEM((D,), BF),
            pltpu.VMEM((D,), BF),
            pltpu.SMEM((1,), I32),
            pltpu.SemaphoreType.DMA((NX + 4,)),
            pltpu.SemaphoreType.DMA((1,)),
        ],
        compiler_params=pltpu.CompilerParams(vmem_limit_bytes=120 * 1024 * 1024),
        name="gated_mix",
    )(A_x, A_wqkv, A_wo, B_w1, B_b1, B_w2, B_b2, gate_w)
```

```python
import math

import jax
import jax.numpy as jnp
from jax import lax
import jax.experimental.pallas as pl
import jax.experimental.pallas.tpu as pltpu

S, D, H, DH, F = 2048, 640, 32, 20, 1536
BF = jnp.bfloat16
F32 = jnp.float32
I32 = jnp.int32

VR = 24
TQ = 512
C = 128
NQ = S // TQ
NC = S // C
NL = TQ // 128
GH = 4
NGRP = H // GH
TF = S // NGRP
NT = 4
T0 = NC - NT
R0 = 16 * NC
R = R0 + 8 * NT
KX = S // 2
ORDER = [0, 1, 2, 12, 3, 4, 5, 13, 6, 7, 8, 14, 9, 10, 11, 15]
TE = 128
NE = S // TE
SFM = 32
X0, XM, NXM = 128, 384, 3
XL = X0 + NXM * XM
NX = NXM + 2
QSCALE = (DH ** -0.5) * math.log2(math.e)
SCORE_BOUND = 60.0
V_HI, V_LO = 2.0 ** 40, 2.0 ** -40
assert NQ == 4 and NL == 4


def _mxu_pieces():
    per_tile = []
    for c in ORDER:
        ps = [(c * 64 + 8 * g, [(c, 16 * g, 16)]) for g in range(7, 0 if c < T0 else 1, -1)]
        if c >= T0 and (c - T0) % 2 == 0:
            ps.append((KX + 4 * (c - T0), [(c, 24, 8), (c + 1, 24, 8)]))
        per_tile.append(ps)
    flat = [p for ps in per_tile for p in ps]
    starts = [sum(len(ps) for ps in per_tile[:n]) for n in range(NC)]
    return flat, [min(len(flat), s + 8) for s in starts], 8 - len(per_tile[-1])


_FLAT, _ENDS, _LA = _mxu_pieces()


def _kernel(x_hbm, wqkv_hbm, wo_hbm, w1_hbm, b1_hbm, w2_hbm, b2_hbm, gw_hbm, o_hbm,
            x_ref, wqkv_ref, wo_ref, w1_ref, w2_ref, o_ref,
            wqvT_ref, kn_ref, k_ref, qp_ref, q32_ref, vT_ref, oT_ref, c_ref, g_ref,
            kf_ref, kb_ref, qb_ref, s_ref, on_ref, qmax_ref, kmax_ref, vmax_ref,
            b1_ref, b2_ref, gw_ref, z_ref, sem_in, sem_out):
    def al(v, m):
        return v if isinstance(v, int) else pl.multiple_of(v, m)

    def true_mask(shape):
        return lax.broadcasted_iota(I32, shape, len(shape) - 1) >= z_ref[0]

    def cp_x(i, lo, n):
        return pltpu.make_async_copy(x_hbm.at[0, pl.ds(lo, n), :], x_ref.at[pl.ds(lo, n), :], sem_in.at[i])

    def cp_xm(i):
        return cp_x(1 + i, al(X0 + i * XM, 128), XM)

    def cp_w(j):
        return pltpu.make_async_copy(wqkv_hbm.at[:, pl.ds(j * D, D)], wqkv_ref.at[j], sem_in.at[NX + j])

    cp_gw = pltpu.make_async_copy(gw_hbm, gw_ref, sem_in.at[0])
    cp_x0 = cp_x(0, 0, X0)
    cp_xl = cp_x(NX - 1, XL, S - XL)
    late = [pltpu.make_async_copy(src, dst, sem_in.at[NX + 3])
            for src, dst in [(w1_hbm, w1_ref), (w2_hbm, w2_ref), (wo_hbm, wo_ref),
                             (b1_hbm, b1_ref), (b2_hbm, b2_ref)]]
    cp_gw.start()
    cp_x0.start()
    cp_w(1).start()
    for i in range(NXM):
        cp_xm(i).start()
    cp_w(0).start()
    cp_w(2).start()
    cp_xl.start()
    for cp in late:
        cp.start()
    z_ref[0] = 0

    def lane_window(slabs, start, lane):
        j, o = divmod(start, 128)
        if o == 0:
            return slabs[j]
        a = slabs[j]
        if j + 1 < len(slabs):
            a = jnp.where(lane >= o, a, slabs[j + 1])
        return pltpu.roll(a, 128 - o, 1)

    def kproj(lo, n, first=False):
        km = None if first else kmax_ref[...]
        gw = gw_ref[...].astype(F32).reshape(1, D)
        lane = lax.broadcasted_iota(I32, (16, 128), 1)
        k = None
        for i in range(n // 128):
            r = lo + i * 128
            xt = x_ref[pl.ds(al(r, 128), 128), :]
            xg = xt.astype(F32)
            if k is not None:
                xg = jnp.where(true_mask((128, D)), xg, k)
            zz = jnp.sum(xg * gw, axis=-1, keepdims=True)
            g_ref[pl.ds(al(r, 128), 128), :] = jnp.broadcast_to(jax.nn.sigmoid(zz), (128, 128))
            k = jnp.dot(xt, wqkv_ref[1], preferred_element_type=F32)
            kn_ref[pl.ds(al(r >> 1, 64), 64), :] = pltpu.bitcast(k.astype(BF), I32)
            kr = jnp.max(jnp.abs(k).reshape(16, 8, D), axis=0)
            km = kr if km is None else jnp.maximum(km, kr)
            slabs = [k[0:16, 128 * j:128 * j + 128] for j in range(D // 128)]
            rows = pl.ds(al(r >> 3, 16), 16)
            for gi in range(NGRP):
                kf_ref[gi, rows, :] = lane_window(slabs, gi * GH * DH, lane)
            if isinstance(r, int) and r // C >= T0:
                u = r // C - T0
                if u % 2 == 0:
                    k_prev = k[16:32]
                else:
                    kx = jnp.concatenate([k_prev[8:16], k[24:32]], axis=0)
                    kn_ref[KX + 8 * (u // 2):KX + 8 * (u // 2) + 8, :] = pltpu.bitcast(kx.astype(BF), I32)
                    ku = jnp.concatenate([k_prev[0:8], k[16:24]], axis=0)
                    slabs = [ku[:, 128 * j:128 * j + 128] for j in range(D // 128)]
                    for gi in range(NGRP):
                        kf_ref[gi, R0 + 8 * (u - 1):R0 + 8 * (u + 1), :] = lane_window(slabs, gi * GH * DH, lane)
        kmax_ref[...] = km

    cp_gw.wait()
    cp_x0.wait()
    cp_w(1).wait()
    kproj(0, X0, first=True)

    def kproj_mid(i, carry):
        cp_xm(i).wait()
        kproj(X0 + i * XM, XM)
        return carry

    lax.fori_loop(0, NXM, kproj_mid, 0)
    cp_w(0).wait()
    cp_w(2).wait()
    cp_xl.wait()
    wqvT_ref[0:D, :] = wqkv_ref[0].T
    wqvT_ref[D:2 * D, :] = wqkv_ref[2].T
    kproj(XL, S - XL)
    qmax_ref[...] = jnp.zeros_like(qmax_ref)
    vmax_ref[...] = jnp.zeros_like(vmax_ref)

    def qvproj(t, carry):
        xt = x_ref[pl.ds(pl.multiple_of(t * TQ, TQ), TQ), :]
        qv = lax.dot_general(wqvT_ref[...], xt, (((1,), (1,)), ((), ())), preferred_element_type=F32)
        qf = qv[:D] * QSCALE
        q32_ref[t] = qf
        v = qv[D:]
        vmax_ref[...] = jnp.maximum(vmax_ref[...], jnp.max(jnp.abs(v).reshape(D // 8, 8, TQ), axis=0))
        row = lax.broadcasted_iota(I32, (VR, TQ), 0)
        zpad = jnp.zeros((32 - VR, TQ), F32)
        qm = qmax_ref[...]
        for h in range(H):
            off = 4 * (h % 2)
            w = h * DH - off
            used = (row >= off) & (row < off + DH)
            qw = jnp.where(used, qf[w:w + VR], 0.0)
            qm = jnp.maximum(qm, jnp.sum((qw * qw).reshape(VR // 8, 8, TQ), axis=0))
            qp_ref[t, h] = pltpu.bitcast(jnp.concatenate([qw, zpad], axis=0).astype(BF), I32)
            vT_ref[t, h] = jnp.where(used, v[w:w + VR], 1.0)
        qmax_ref[...] = qm
        rk = pl.multiple_of(t * (TQ // 2), TQ // 2)
        tx = jnp.minimum(t, NT // 2 - 1)
        rx = pl.multiple_of(KX + 8 * tx, 8)
        kn = jnp.concatenate([kn_ref[pl.ds(rk, TQ // 2), :], kn_ref[pl.ds(rx, 8), :]], axis=0)
        slabs = [kn[:, 128 * j:128 * j + 128] for j in range(D // 128)]
        lane = lax.broadcasted_iota(I32, (TQ // 2 + 8, 128), 1)
        for h in range(H):
            j, o = divmod(h * DH - 4 * (h % 2), 128)
            sl = slabs[j:j + 2] if o + 32 > 128 else slabs[j:j + 1]
            kw = lane_window(sl, o, lane)
            k_ref[h, pl.ds(rk, TQ // 2), :] = kw[:TQ // 2]
            k_ref[h, pl.ds(rx, 8), :] = kw[TQ // 2:]
        nr = R0 // NQ
        rr = pl.ds(pl.multiple_of(t * nr, nr), nr)
        re = pl.ds(pl.multiple_of(R0 + 16 * tx, 16), 16)
        for ln in range(GH * DH):
            hh, d = divmod(ln, DH)
            kb_ref[hh, d, rr, :] = jnp.broadcast_to(kf_ref[0, rr, ln:ln + 1], (nr, 128))
            kb_ref[hh, d, re, :] = jnp.broadcast_to(kf_ref[0, re, ln:ln + 1], (16, 128))
            bq = jnp.broadcast_to(qf[ln:ln + 1], (8, TQ))
            for j in range(NL):
                qb_ref[hh, t, d, j] = bq[:, 128 * j:128 * j + 128]
        return carry

    lax.fori_loop(0, NQ, qvproj, 0)
    for cp in late:
        cp.wait()

    qn2 = jnp.sum(jnp.max(qmax_ref[...], axis=1, keepdims=True), axis=0, keepdims=True)
    ka = jnp.max(kmax_ref[...], axis=0, keepdims=True)
    rel = lax.broadcasted_iota(I32, (H, D), 1) - DH * lax.broadcasted_iota(I32, (H, D), 0)
    kn2 = jnp.sum(jnp.where((rel >= 0) & (rel < DH), ka * ka, 0.0), axis=1, keepdims=True)
    kn2 = jnp.max(kn2, axis=0, keepdims=True)
    vm = jnp.max(jnp.max(vmax_ref[...], axis=0, keepdims=True), axis=1, keepdims=True)
    safe = (qn2 * kn2 <= SCORE_BOUND * SCORE_BOUND) & (vm <= V_HI) & (vm >= V_LO)
    unsafe = jnp.max(jnp.where(safe, 0, 1).astype(I32))

    def finish(h, odd, qb, acc):
        off = odd * 4
        l = jnp.where(odd == 1, acc[0:1], acc[VR - 1:VR])
        row = lax.broadcasted_iota(I32, (VR, TQ), 0)
        used = (row >= off) & (row < off + DH)
        pltpu.store(oT_ref.at[qb, pl.ds(pl.multiple_of(h * DH - off, 8), VR), :], acc * (1.0 / l), mask=used)

    def ffn_rows(i, n, mid=None):
        r0 = pl.multiple_of(i * n, n)
        hid = jnp.dot(x_ref[pl.ds(r0, n), :], w1_ref[...], preferred_element_type=F32)
        hid = hid + b1_ref[...].astype(F32).reshape(1, F)
        if mid is not None:
            mid()
        r = jnp.maximum(hid, 0.0)
        b = jnp.dot((r * r).astype(BF), w2_ref[...], preferred_element_type=F32)
        b = b + b2_ref[...].astype(F32).reshape(1, D)
        g = g_ref[pl.ds(r0, n), :]
        c_ref[pl.ds(r0, n), :] = (1.0 - jnp.concatenate([g] * (D // 128), axis=1)) * b

    def fast_group(gi, carry):
        h0 = gi * GH
        link = {n: true_mask((1, n, 128)) for n in (16, 24)}

        def ids(it):
            hh, qb = it >> 2, it & 3
            return hh, qb, h0 + hh

        def mxu_scores(idx, lo, hi, parts):
            _, qb, h = idx
            kk = pltpu.bitcast(jnp.concatenate([k_ref[h, r:r + 8, :] for r, _ in _FLAT[lo:hi]], axis=0), BF)
            e = jnp.exp2(jnp.dot(kk[:, :32], pltpu.bitcast(qp_ref[qb, h], BF), preferred_element_type=F32))
            r = 0
            for _, dests in _FLAT[lo:hi]:
                for c, row, n in dests:
                    parts[(c, row)] = e[r:r + n]
                    r += n

        def vpu_scores(idx, c, parts, chain):
            hh, qb, _ = idx
            nk = 16 if c < T0 else 24
            res = []
            for j in range(NL):
                kv = kb_ref[hh, :, 16 * c:16 * c + 16, :]
                if c >= T0:
                    kv = jnp.concatenate([kv, kb_ref[hh, :, R0 + 8 * (c - T0):R0 + 8 * (c - T0 + 1), :]], axis=1)
                pr = (kv.reshape(DH, nk // 8, 8, 128) * qb_ref[hh, qb, :, j:j + 1]).reshape(DH, nk, 128)
                if c < T0:
                    pr = pr.reshape(2, 10, nk, 128)
                    t = pr[:, 1:].reshape(2, 3, 3, nk, 128)
                    t = jnp.concatenate([t[:, :, 0:1], t[:, :, 1:2] + t[:, :, 2:3]], axis=2)
                    pr = jnp.concatenate([pr[:, 0:1], t.reshape(2, 6, nk, 128)], axis=1).reshape(14, nk, 128)
                if chain is not None:
                    if chain.shape[1] < nk:
                        chain = jnp.concatenate([chain, chain[:, :8]], axis=1)
                    pr = jnp.concatenate([jnp.where(link[nk], pr[0:1], chain[:, :nk]), pr[1:]], axis=0)
                chain = jnp.sum(pr, axis=0, keepdims=True)
                res.append(chain[0])
            parts[(c, 0)] = jnp.exp2(jnp.concatenate(res, axis=1))
            return chain

        def tile(parts, n):
            return jnp.concatenate([parts.pop(k) for k in sorted(parts) if k[0] == ORDER[n]], axis=0)

        def pv(idx, n, p):
            t, lo = divmod(ORDER[n] * C, TQ)
            return jnp.dot(vT_ref[t, idx[2], :, lo:lo + C], p, preferred_element_type=F32)

        def close(it, p, acc):
            idx = ids(it)
            finish(idx[2], idx[0] & 1, idx[1], pv(idx, NC - 1, p) + acc)

        def item(it, state):
            chain, p14, p15, acc_prev = state
            idx = ids(it)
            parts = {}
            lo = 0
            if p14 is not None:
                mxu_scores(idx, 0, _LA, parts)
                lo = _LA
                acc_prev = pv(ids(it - 1), NC - 2, p14) + acc_prev
            acc = None
            for n in range(NC):
                mxu_scores(idx, lo, _ENDS[n], parts)
                lo = _ENDS[n]
                chain = vpu_scores(idx, ORDER[n], parts, chain)
                if n == 0 and p14 is not None:
                    close(it - 1, p15, acc_prev)
                if 0 < n < NC - 1:
                    o = pv(idx, n - 1, tile(parts, n - 1))
                    acc = o if acc is None else o + acc
            return chain, tile(parts, NC - 2), tile(parts, NC - 1), acc

        state = item(0, (None, None, None, None))
        _, p14, p15, acc_last = lax.fori_loop(1, GH * NQ, item, state, unroll=True)
        acc_last = pv(ids(GH * NQ - 1), NC - 2, p14) + acc_last
        ffn_rows(gi, TF, mid=lambda: close(GH * NQ - 1, p15, acc_last))

        gn = jnp.minimum(gi + 1, NGRP - 1)
        pace = true_mask((NQ, NL, 8, 128))
        for ln in range(GH * DH):
            hh, d = divmod(ln, DH)
            kbv = jnp.broadcast_to(kf_ref[gn][:, ln:ln + 1], (R, 128))
            kb_ref[hh, d, 0:R, :] = kbv
            qw = q32_ref[:, pl.ds(pl.multiple_of(gn * (GH * DH) + ln // 8 * 8, 8), 8), :]
            bq = jnp.broadcast_to(qw[:, ln % 8:ln % 8 + 1, :], (NQ, 8, TQ))
            bq = jnp.stack([bq[:, :, 128 * j:128 * j + 128] for j in range(NL)], axis=1)
            tie = kbv[:R0].reshape(NQ, NL, 16, 128)[:, :, 0:8]
            qb_ref[hh, :, d, 0:NL] = jnp.where(pace, bq, tie)
        return carry

    def fast_path():
        lax.fori_loop(0, NGRP, fast_group, 0)

    def slow_ffn(i, carry):
        ffn_rows(i, SFM)
        return carry

    def slow_item(i, carry):
        h, qb = i >> 2, i & 3

        def pass1(t, mx):
            kk = pltpu.bitcast(k_ref[h, pl.ds(pl.multiple_of(t * (TQ // 2), TQ // 2), TQ // 2), :], BF)[:, :32]
            s = jnp.dot(kk, pltpu.bitcast(qp_ref[qb, h], BF), preferred_element_type=F32)
            s_ref[t] = s
            return jnp.maximum(mx, jnp.max(s.reshape(TQ // 8, 8, TQ), axis=0))

        mx = lax.fori_loop(0, NQ, pass1, jnp.full((8, TQ), -jnp.inf, F32))
        m = jnp.max(mx, axis=0, keepdims=True)

        def pass2(t, acc):
            p = jnp.exp2(s_ref[t] - m).astype(BF)
            return acc + jnp.dot(vT_ref[t, h], p, preferred_element_type=F32)

        finish(h, h & 1, qb, lax.fori_loop(0, NQ, pass2, jnp.zeros((VR, TQ), F32)))
        return carry

    def slow_path():
        lax.fori_loop(0, S // SFM, slow_ffn, 0)
        lax.fori_loop(0, H * NQ, slow_item, 0)

    lax.cond(unsafe == 0, fast_path, slow_path)

    def cp_out(e):
        r0 = al(e * TE, TE)
        return pltpu.make_async_copy(o_ref.at[pl.ds(r0, TE), :], o_hbm.at[0, pl.ds(r0, TE), :], sem_out.at[0])

    def o_chunk(qb, sub):
        return oT_ref[qb, :, sub * TE:(sub + 1) * TE].T.astype(BF)

    def epilogue(qb, carry):
        for sub in range(TQ // TE):
            e = qb * (TQ // TE) + sub
            r0 = pl.multiple_of(e * TE, TE)
            o = pltpu.bitcast(on_ref[...], BF) if sub == 0 else o_chunk(qb, sub)
            a = jnp.dot(o, wo_ref[...], preferred_element_type=F32)
            g = jnp.concatenate([g_ref[pl.ds(r0, TE), :]] * (D // 128), axis=1)
            o_ref[pl.ds(r0, TE), :] = (g * a + c_ref[pl.ds(r0, TE), :]).astype(o_ref.dtype)
            cp_out(e).start()
        on_ref[...] = pltpu.bitcast(o_chunk(jnp.minimum(qb + 1, NQ - 1), 0), I32)
        return carry

    on_ref[...] = pltpu.bitcast(o_chunk(0, 0), I32)
    lax.fori_loop(0, NQ, epilogue, 0)
    for e in range(NE):
        cp_out(e).wait()


@jax.jit
def pallas_gated_mix__softmax_full_mha__dense_activation_squared_relu__prompt_kernel(
    A_x: jax.Array,
    A_wqkv: jax.Array,
    A_wo: jax.Array,
    B_x: jax.Array,
    B_w1: jax.Array,
    B_b1: jax.Array,
    B_w2: jax.Array,
    B_b2: jax.Array,
    gate_w: jax.Array,
):
    del B_x
    hbm = pl.BlockSpec(memory_space=pl.ANY)
    return pl.pallas_call(
        _kernel,
        in_specs=[hbm] * 8,
        out_specs=hbm,
        out_shape=jax.ShapeDtypeStruct((1, S, D), BF),
        scratch_shapes=[
            pltpu.VMEM((S, D), BF),
            pltpu.VMEM((3, D, D), BF),
            pltpu.VMEM((D, D), BF),
            pltpu.VMEM((D, F), BF),
            pltpu.VMEM((F, D), BF),
            pltpu.VMEM((S, D), BF),
            pltpu.VMEM((2 * D, D), BF),
            pltpu.VMEM((KX + 128, D), I32),
            pltpu.VMEM((H, KX + 32, 128), I32),
            pltpu.VMEM((NQ, H, 16, TQ), I32),
            pltpu.VMEM((NQ, D, TQ), F32),
            pltpu.VMEM((NQ, H, VR, TQ), F32),
            pltpu.VMEM((NQ, D, TQ), F32),
            pltpu.VMEM((S, D), F32),
            pltpu.VMEM((S, 128), F32),
            pltpu.VMEM((NGRP, R, 128), F32),
            pltpu.VMEM((GH, DH, R + 8, 128), F32),
            pltpu.VMEM((GH, NQ, DH, NL + 1, 8, 128), F32),
            pltpu.VMEM((NQ, TQ, TQ), F32),
            pltpu.VMEM((TE // 2, D), I32),
            pltpu.VMEM((8, TQ), F32),
            pltpu.VMEM((8, D), F32),
            pltpu.VMEM((8, TQ), F32),
            pltpu.VMEM((F,), BF),
            pltpu.VMEM((D,), BF),
            pltpu.VMEM((D,), BF),
            pltpu.SMEM((1,), I32),
            pltpu.SemaphoreType.DMA((NX + 4,)),
            pltpu.SemaphoreType.DMA((1,)),
        ],
        compiler_params=pltpu.CompilerParams(vmem_limit_bytes=120 * 1024 * 1024),
        name="gated_mix",
    )(A_x, A_wqkv, A_wo, B_w1, B_b1, B_w2, B_b2, gate_w)
```

```python
import math

import jax
import jax.numpy as jnp
from jax import lax
import jax.experimental.pallas as pl
import jax.experimental.pallas.tpu as pltpu

S, D, H, DH, F = 2048, 640, 32, 20, 1536
BF = jnp.bfloat16
F32 = jnp.float32
I32 = jnp.int32

VR = 24
TQ = 512
C = 128
NQ = S // TQ
NC = S // C
NL = TQ // 128
GH = 4
NGRP = H // GH
TF = S // NGRP
NT = 4
T0 = NC - NT
R0 = 16 * NC
R = R0 + 8 * NT
KX = S // 2
ORDER = [0, 1, 2, 12, 3, 4, 5, 13, 6, 7, 8, 14, 9, 10, 11, 15]
MC = 256
TE = 128
NE = S // TE
SFM = 32
X0, XM, NXM = 128, 384, 3
XL = X0 + NXM * XM
NX = NXM + 2
QSCALE = (DH ** -0.5) * math.log2(math.e)
SCORE_BOUND = 60.0
V_HI, V_LO = 2.0 ** 40, 2.0 ** -40
assert NQ == 4 and NL == 4 and NT == NQ and XL <= T0 * C


def _mxu_pieces():
    per_tile = []
    for c in ORDER:
        ps = [(c * 64 + 8 * g, [(c, 16 * g, 16)]) for g in range(7, 0 if c < T0 else 1, -1)]
        if c >= T0 and (c - T0) % 2 == 0:
            ps.append((KX + 4 * (c - T0), [(c, 24, 8), (c + 1, 24, 8)]))
        per_tile.append(ps)
    flat = [p for ps in per_tile for p in ps]
    starts = [sum(len(ps) for ps in per_tile[:n]) for n in range(NC)]
    return flat, [min(len(flat), s + 8) for s in starts], 8 - len(per_tile[-1])


_FLAT, _ENDS, _LA = _mxu_pieces()


def _kernel(x_hbm, wqkv_hbm, wo_hbm, w1_hbm, b1_hbm, w2_hbm, b2_hbm, gw_hbm, o_hbm,
            x_ref, wqkv_ref, wo_ref, w1_ref, w2_ref, o_ref,
            wqvT_ref, kn_ref, k_ref, qp_ref, q32_ref, vT_ref, oT_ref, c_ref, g_ref,
            kf_ref, kb_ref, qb_ref, s_ref, on_ref, qmax_ref, kmax_ref, vmax_ref,
            b1_ref, b2_ref, gw_ref, z_ref, sem_in, sem_out):
    def al(v, m):
        return v if isinstance(v, int) else pl.multiple_of(v, m)

    def true_mask(shape):
        return lax.broadcasted_iota(I32, shape, len(shape) - 1) >= z_ref[0]

    def cp_x(i, lo, n):
        return pltpu.make_async_copy(x_hbm.at[0, pl.ds(lo, n), :], x_ref.at[pl.ds(lo, n), :], sem_in.at[i])

    def cp_xm(i):
        return cp_x(1 + i, al(X0 + i * XM, 128), XM)

    def cp_w(j):
        return pltpu.make_async_copy(wqkv_hbm.at[:, pl.ds(j * D, D)], wqkv_ref.at[j], sem_in.at[NX + j])

    cp_gw = pltpu.make_async_copy(gw_hbm, gw_ref, sem_in.at[0])
    cp_x0 = cp_x(0, 0, X0)
    cp_xl = cp_x(NX - 1, XL, S - XL)
    late = [pltpu.make_async_copy(src, dst, sem_in.at[NX + 3])
            for src, dst in [(w1_hbm, w1_ref), (w2_hbm, w2_ref), (wo_hbm, wo_ref),
                             (b1_hbm, b1_ref), (b2_hbm, b2_ref)]]
    cp_gw.start()
    cp_x0.start()
    cp_w(1).start()
    for i in range(NXM):
        cp_xm(i).start()
    cp_w(0).start()
    cp_w(2).start()
    cp_xl.start()
    for cp in late:
        cp.start()
    z_ref[0] = 0

    def lane_window(slabs, start, lane):
        j, o = divmod(start, 128)
        if o == 0:
            return slabs[j]
        a = slabs[j]
        if j + 1 < len(slabs):
            a = jnp.where(lane >= o, a, slabs[j + 1])
        return pltpu.roll(a, 128 - o, 1)

    def kproj(lo, n, first=False):
        km = None if first else kmax_ref[...]
        gw = gw_ref[...].astype(F32).reshape(1, D)
        lane = lax.broadcasted_iota(I32, (16, 128), 1)
        k = None
        for i in range(n // 128):
            r = lo + i * 128
            xt = x_ref[pl.ds(al(r, 128), 128), :]
            xg = xt.astype(F32)
            if k is not None:
                xg = jnp.where(true_mask((128, D)), xg, k)
            zz = jnp.sum(xg * gw, axis=-1, keepdims=True)
            g_ref[pl.ds(al(r, 128), 128), :] = jnp.broadcast_to(jax.nn.sigmoid(zz), (128, 128))
            k = jnp.dot(xt, wqkv_ref[1], preferred_element_type=F32)
            kn_ref[pl.ds(al(r >> 1, 64), 64), :] = pltpu.bitcast(k.astype(BF), I32)
            kr = jnp.max(jnp.abs(k).reshape(16, 8, D), axis=0)
            km = kr if km is None else jnp.maximum(km, kr)
            slabs = [k[0:16, 128 * j:128 * j + 128] for j in range(D // 128)]
            rows = pl.ds(al(r >> 3, 16), 16)
            for gi in range(NGRP):
                kf_ref[gi, rows, :] = lane_window(slabs, gi * GH * DH, lane)
            if isinstance(r, int) and r // C >= T0:
                u = r // C - T0
                if u % 2 == 0:
                    k_prev = k[16:32]
                else:
                    kx = jnp.concatenate([k_prev[8:16], k[24:32]], axis=0)
                    kn_ref[KX + 8 * (u // 2):KX + 8 * (u // 2) + 8, :] = pltpu.bitcast(kx.astype(BF), I32)
                    ku = jnp.concatenate([k_prev[0:8], k[16:24]], axis=0)
                    slabs = [ku[:, 128 * j:128 * j + 128] for j in range(D // 128)]
                    for gi in range(NGRP):
                        kf_ref[gi, R0 + 8 * (u - 1):R0 + 8 * (u + 1), :] = lane_window(slabs, gi * GH * DH, lane)
        kmax_ref[...] = km

    cp_gw.wait()
    cp_x0.wait()
    cp_w(1).wait()
    kproj(0, X0, first=True)

    def kproj_mid(i, carry):
        cp_xm(i).wait()
        kproj(X0 + i * XM, XM)
        return carry

    lax.fori_loop(0, NXM, kproj_mid, 0)
    cp_w(0).wait()
    cp_w(2).wait()
    cp_xl.wait()
    wqvT_ref[0:D, :] = wqkv_ref[0].T
    wqvT_ref[D:2 * D, :] = wqkv_ref[2].T
    kproj(XL, S - XL)
    qmax_ref[...] = jnp.zeros_like(qmax_ref)
    vmax_ref[...] = jnp.zeros_like(vmax_ref)

    def qvproj(t, carry):
        xt = x_ref[pl.ds(pl.multiple_of(t * TQ, TQ), TQ), :]
        qv = jnp.concatenate([lax.dot_general(wqvT_ref[m:m + MC, :], xt, (((1,), (1,)), ((), ())), preferred_element_type=F32)
                              for m in range(0, 2 * D, MC)], axis=0)
        qf = qv[:D] * QSCALE
        q32_ref[t] = qf
        v = qv[D:]
        vmax_ref[...] = jnp.maximum(vmax_ref[...], jnp.max(jnp.abs(v).reshape(D // 8, 8, TQ), axis=0))
        row = lax.broadcasted_iota(I32, (VR, TQ), 0)
        zpad = jnp.zeros((32 - VR, TQ), F32)
        qm = qmax_ref[...]
        for h in range(H):
            off = 4 * (h % 2)
            w = h * DH - off
            used = (row >= off) & (row < off + DH)
            qw = jnp.where(used, qf[w:w + VR], 0.0)
            qm = jnp.maximum(qm, jnp.sum((qw * qw).reshape(VR // 8, 8, TQ), axis=0))
            qp_ref[t, h] = pltpu.bitcast(jnp.concatenate([qw, zpad], axis=0).astype(BF), I32)
            vT_ref[t, h] = jnp.where(used, v[w:w + VR], 1.0)
        qmax_ref[...] = qm
        rk = pl.multiple_of(t * (TQ // 2), TQ // 2)
        rx = pl.multiple_of(KX + 8 * (t >> 1), 8)
        kn = jnp.concatenate([kn_ref[pl.ds(rk, TQ // 2), :], kn_ref[pl.ds(rx, 8), :]], axis=0)
        slabs = [kn[:, 128 * j:128 * j + 128] for j in range(D // 128)]
        lane = lax.broadcasted_iota(I32, (TQ // 2 + 8, 128), 1)
        for h in range(H):
            j, o = divmod(h * DH - 4 * (h % 2), 128)
            sl = slabs[j:j + 2] if o + 32 > 128 else slabs[j:j + 1]
            kw = lane_window(sl, o, lane)
            k_ref[h, pl.ds(rk, TQ // 2), :] = kw[:TQ // 2]
            k_ref[h, pl.ds(rx, 8), :] = kw[TQ // 2:]
        nr = R0 // NQ
        rr = pl.ds(pl.multiple_of(t * nr, nr), nr)
        re = pl.ds(pl.multiple_of(R0 + 8 * t, 8), 8)
        kf = jnp.concatenate([kf_ref[0, rr, :], kf_ref[0, re, :]], axis=0)
        for ln in range(GH * DH):
            hh, d = divmod(ln, DH)
            kbv = jnp.broadcast_to(kf[:, ln:ln + 1], (nr + 8, 128))
            kb_ref[hh, d, rr, :] = kbv[:nr]
            kb_ref[hh, d, re, :] = kbv[nr:]
            bq = jnp.broadcast_to(qf[ln:ln + 1], (8, TQ))
            qb_ref[hh, t, d, 0:NL] = jnp.stack([bq[:, 128 * j:128 * j + 128] for j in range(NL)], axis=0)
        return carry

    lax.fori_loop(0, NQ, qvproj, 0)
    for cp in late:
        cp.wait()

    qn2 = jnp.sum(jnp.max(qmax_ref[...], axis=1, keepdims=True), axis=0, keepdims=True)
    ka = jnp.max(kmax_ref[...], axis=0, keepdims=True)
    rel = lax.broadcasted_iota(I32, (H, D), 1) - DH * lax.broadcasted_iota(I32, (H, D), 0)
    kn2 = jnp.sum(jnp.where((rel >= 0) & (rel < DH), ka * ka, 0.0), axis=1, keepdims=True)
    kn2 = jnp.max(kn2, axis=0, keepdims=True)
    vm = jnp.max(jnp.max(vmax_ref[...], axis=0, keepdims=True), axis=1, keepdims=True)
    safe = (qn2 * kn2 <= SCORE_BOUND * SCORE_BOUND) & (vm <= V_HI) & (vm >= V_LO)
    unsafe = jnp.max(jnp.where(safe, 0, 1).astype(I32))

    def finish(h, odd, qb, acc):
        off = odd * 4
        l = jnp.where(odd == 1, acc[0:1], acc[VR - 1:VR])
        row = lax.broadcasted_iota(I32, (VR, TQ), 0)
        used = (row >= off) & (row < off + DH)
        pltpu.store(oT_ref.at[qb, pl.ds(pl.multiple_of(h * DH - off, 8), VR), :], acc * (1.0 / l), mask=used)

    def ffn_rows(i, n, mid=None):
        r0 = pl.multiple_of(i * n, n)
        hid = jnp.dot(x_ref[pl.ds(r0, n), :], w1_ref[...], preferred_element_type=F32)
        hid = hid + b1_ref[...].astype(F32).reshape(1, F)
        if mid is not None:
            mid()
        r = jnp.maximum(hid, 0.0)
        b = jnp.dot((r * r).astype(BF), w2_ref[...], preferred_element_type=F32)
        b = b + b2_ref[...].astype(F32).reshape(1, D)
        g = g_ref[pl.ds(r0, n), :]
        c_ref[pl.ds(r0, n), :] = (1.0 - jnp.concatenate([g] * (D // 128), axis=1)) * b

    def fast_group(gi, carry):
        h0 = gi * GH
        link = {n: true_mask((1, n, 128)) for n in (16, 24)}

        def ids(it):
            hh, qb = it >> 2, it & 3
            return hh, qb, h0 + hh

        def mxu_scores(idx, lo, hi, parts):
            _, qb, h = idx
            rows = [r for r, _ in _FLAT[lo:hi]]
            kt = {}
            for b in sorted({r // 64 for r in rows}):
                r0, r1 = min(r for r in rows if r // 64 == b), max(r for r in rows if r // 64 == b) + 8
                kt[b] = (r0, k_ref[h, r0:r1, :])
            kk = jnp.concatenate([kt[r // 64][1][r - kt[r // 64][0]:r - kt[r // 64][0] + 8] for r in rows], axis=0)
            kk = pltpu.bitcast(kk, BF)
            e = jnp.exp2(jnp.dot(kk[:, :32], pltpu.bitcast(qp_ref[qb, h], BF), preferred_element_type=F32))
            r = 0
            for _, dests in _FLAT[lo:hi]:
                for c, row, n in dests:
                    parts[(c, row)] = e[r:r + n]
                    r += n

        def vpu_scores(idx, c, parts, chain):
            hh, qb, _ = idx
            nk = 16 if c < T0 else 24
            res = []
            for j in range(NL):
                kv = kb_ref[hh, :, 16 * c:16 * c + 16, :]
                if c >= T0:
                    kv = jnp.concatenate([kv, kb_ref[hh, :, R0 + 8 * (c - T0):R0 + 8 * (c - T0 + 1), :]], axis=1)
                pr = (kv.reshape(DH, nk // 8, 8, 128) * qb_ref[hh, qb, :, j:j + 1]).reshape(DH, nk, 128)
                if c < T0:
                    pr = pr.reshape(2, 10, nk, 128)
                    t = pr[:, 1:].reshape(2, 3, 3, nk, 128)
                    t = jnp.concatenate([t[:, :, 0:1], t[:, :, 1:2] + t[:, :, 2:3]], axis=2)
                    pr = jnp.concatenate([pr[:, 0:1], t.reshape(2, 6, nk, 128)], axis=1).reshape(14, nk, 128)
                if chain is not None:
                    if chain.shape[1] < nk:
                        chain = jnp.concatenate([chain, chain[:, :8]], axis=1)
                    pr = jnp.concatenate([jnp.where(link[nk], pr[0:1], chain[:, :nk]), pr[1:]], axis=0)
                chain = jnp.sum(pr, axis=0, keepdims=True)
                res.append(chain[0])
            parts[(c, 0)] = jnp.exp2(jnp.concatenate(res, axis=1))
            return chain

        def tile(parts, n):
            return jnp.concatenate([parts.pop(k) for k in sorted(parts) if k[0] == ORDER[n]], axis=0)

        def pv(idx, n, p):
            t, lo = divmod(ORDER[n] * C, TQ)
            return jnp.dot(vT_ref[t, idx[2], :, lo:lo + C], p, preferred_element_type=F32)

        def close(it, p, acc):
            idx = ids(it)
            finish(idx[2], idx[0] & 1, idx[1], pv(idx, NC - 1, p) + acc)

        def item(it, state):
            chain, p14, p15, acc_prev = state
            idx = ids(it)
            parts = {}
            lo = 0
            if p14 is not None:
                mxu_scores(idx, 0, _LA, parts)
                lo = _LA
                acc_prev = pv(ids(it - 1), NC - 2, p14) + acc_prev
            acc = None
            for n in range(NC):
                mxu_scores(idx, lo, _ENDS[n], parts)
                lo = _ENDS[n]
                chain = vpu_scores(idx, ORDER[n], parts, chain)
                if n == 0 and p14 is not None:
                    close(it - 1, p15, acc_prev)
                if 0 < n < NC - 1:
                    o = pv(idx, n - 1, tile(parts, n - 1))
                    acc = o if acc is None else o + acc
            return chain, tile(parts, NC - 2), tile(parts, NC - 1), acc

        state = item(0, (None, None, None, None))
        _, p14, p15, acc_last = lax.fori_loop(1, GH * NQ, item, state, unroll=True)
        acc_last = pv(ids(GH * NQ - 1), NC - 2, p14) + acc_last
        ffn_rows(2 * gi, TF // 2, mid=lambda: close(GH * NQ - 1, p15, acc_last))
        ffn_rows(2 * gi + 1, TF // 2)

        gn = jnp.minimum(gi + 1, NGRP - 1)
        pace = true_mask((NQ, NL, 8, 128))
        for ln in range(GH * DH):
            hh, d = divmod(ln, DH)
            kbv = jnp.broadcast_to(kf_ref[gn][:, ln:ln + 1], (R, 128))
            kb_ref[hh, d, 0:R, :] = kbv
            qw = q32_ref[:, pl.ds(pl.multiple_of(gn * (GH * DH) + ln // 8 * 8, 8), 8), :]
            bq = jnp.broadcast_to(qw[:, ln % 8:ln % 8 + 1, :], (NQ, 8, TQ))
            bq = jnp.stack([bq[:, :, 128 * j:128 * j + 128] for j in range(NL)], axis=1)
            tie = kbv[:R0].reshape(NQ, NL, 16, 128)[:, :, 0:8]
            qb_ref[hh, :, d, 0:NL] = jnp.where(pace, bq, tie)
        return carry

    def fast_path():
        lax.fori_loop(0, NGRP, fast_group, 0)

    def slow_ffn(i, carry):
        ffn_rows(i, SFM)
        return carry

    def slow_item(i, carry):
        h, qb = i >> 2, i & 3

        def pass1(t, mx):
            kk = pltpu.bitcast(k_ref[h, pl.ds(pl.multiple_of(t * (TQ // 2), TQ // 2), TQ // 2), :], BF)[:, :32]
            s = jnp.dot(kk, pltpu.bitcast(qp_ref[qb, h], BF), preferred_element_type=F32)
            s_ref[t] = s
            return jnp.maximum(mx, jnp.max(s.reshape(TQ // 8, 8, TQ), axis=0))

        mx = lax.fori_loop(0, NQ, pass1, jnp.full((8, TQ), -jnp.inf, F32))
        m = jnp.max(mx, axis=0, keepdims=True)

        def pass2(t, acc):
            p = jnp.exp2(s_ref[t] - m).astype(BF)
            return acc + jnp.dot(vT_ref[t, h], p, preferred_element_type=F32)

        finish(h, h & 1, qb, lax.fori_loop(0, NQ, pass2, jnp.zeros((VR, TQ), F32)))
        return carry

    def slow_path():
        lax.fori_loop(0, S // SFM, slow_ffn, 0)
        lax.fori_loop(0, H * NQ, slow_item, 0)

    lax.cond(unsafe == 0, fast_path, slow_path)

    def cp_out(e):
        r0 = al(e * TE, TE)
        return pltpu.make_async_copy(o_ref.at[pl.ds(r0, TE), :], o_hbm.at[0, pl.ds(r0, TE), :], sem_out.at[0])

    def o_chunk(qb, sub):
        return oT_ref[qb, :, sub * TE:(sub + 1) * TE].T.astype(BF)

    def epilogue(qb, carry):
        for sub in range(TQ // TE):
            e = qb * (TQ // TE) + sub
            r0 = pl.multiple_of(e * TE, TE)
            o = pltpu.bitcast(on_ref[...], BF) if sub == 0 else o_chunk(qb, sub)
            a = jnp.dot(o, wo_ref[...], preferred_element_type=F32)
            g = jnp.concatenate([g_ref[pl.ds(r0, TE), :]] * (D // 128), axis=1)
            o_ref[pl.ds(r0, TE), :] = (g * a + c_ref[pl.ds(r0, TE), :]).astype(o_ref.dtype)
            cp_out(e).start()
        on_ref[...] = pltpu.bitcast(o_chunk(jnp.minimum(qb + 1, NQ - 1), 0), I32)
        return carry

    on_ref[...] = pltpu.bitcast(o_chunk(0, 0), I32)
    lax.fori_loop(0, NQ, epilogue, 0)
    for e in range(NE):
        cp_out(e).wait()


@jax.jit
def pallas_gated_mix__softmax_full_mha__dense_activation_squared_relu__prompt_kernel(
    A_x: jax.Array,
    A_wqkv: jax.Array,
    A_wo: jax.Array,
    B_x: jax.Array,
    B_w1: jax.Array,
    B_b1: jax.Array,
    B_w2: jax.Array,
    B_b2: jax.Array,
    gate_w: jax.Array,
):
    del B_x
    hbm = pl.BlockSpec(memory_space=pl.ANY)
    return pl.pallas_call(
        _kernel,
        in_specs=[hbm] * 8,
        out_specs=hbm,
        out_shape=jax.ShapeDtypeStruct((1, S, D), BF),
        scratch_shapes=[
            pltpu.VMEM((S, D), BF),
            pltpu.VMEM((3, D, D), BF),
            pltpu.VMEM((D, D), BF),
            pltpu.VMEM((D, F), BF),
            pltpu.VMEM((F, D), BF),
            pltpu.VMEM((S, D), BF),
            pltpu.VMEM((2 * D, D), BF),
            pltpu.VMEM((KX + 128, D), I32),
            pltpu.VMEM((H, KX + 32, 128), I32),
            pltpu.VMEM((NQ, H, 16, TQ), I32),
            pltpu.VMEM((NQ, D, TQ), F32),
            pltpu.VMEM((NQ, H, VR, TQ), F32),
            pltpu.VMEM((NQ, D, TQ), F32),
            pltpu.VMEM((S, D), F32),
            pltpu.VMEM((S, 128), F32),
            pltpu.VMEM((NGRP, R, 128), F32),
            pltpu.VMEM((GH, DH, R + 8, 128), F32),
            pltpu.VMEM((GH, NQ, DH, NL + 1, 8, 128), F32),
            pltpu.VMEM((NQ, TQ, TQ), F32),
            pltpu.VMEM((TE // 2, D), I32),
            pltpu.VMEM((8, TQ), F32),
            pltpu.VMEM((8, D), F32),
            pltpu.VMEM((8, TQ), F32),
            pltpu.VMEM((F,), BF),
            pltpu.VMEM((D,), BF),
            pltpu.VMEM((D,), BF),
            pltpu.SMEM((1,), I32),
            pltpu.SemaphoreType.DMA((NX + 4,)),
            pltpu.SemaphoreType.DMA((1,)),
        ],
        compiler_params=pltpu.CompilerParams(vmem_limit_bytes=120 * 1024 * 1024),
        name="gated_mix",
    )(A_x, A_wqkv, A_wo, B_w1, B_b1, B_w2, B_b2, gate_w)
```
